```python
import jax
import jax.numpy as jnp

def _softmax(x, axis=-1):
    return jax.nn.softmax(x, axis=axis)
def _gelu(x):
    return jax.nn.gelu(x, approximate=True)
def _silu(x):
    return jax.nn.silu(x)
def _sigmoid(x):
    return jax.nn.sigmoid(x)
def _layernorm(x, axis=-1, eps=1e-5):
    m = jnp.mean(x, axis=axis, keepdims=True)
    v = jnp.var(x, axis=axis, keepdims=True)
    return (x - m) / jnp.sqrt(v + eps)
def _scatter_add(tgt, idx, src, axis=0):
    return tgt.at[idx].add(src)
def _segment_sum(src, seg, n):
    return jax.ops.segment_sum(src, seg, n)
class _Rng:
    def __init__(self, key):
        self._k = key
    def _next(self):
        self._k, sub = jax.random.split(self._k)
        return sub
    def normal(self, shape):
        return jax.random.normal(self._next(), shape, dtype=jnp.bfloat16)
    def randint(self, lo, hi, shape):
        return jax.random.randint(self._next(), shape, lo, hi, dtype=jnp.int32)
    def uniform(self, shape, lo=0.0, hi=1.0):
        return jax.random.uniform(self._next(), shape, jnp.bfloat16, lo, hi)
    def permutation(self, n):
        return jax.random.permutation(self._next(), n)


kernel_name = 'gated_mix__mha_block_cached__compressed_kv_cla__decode'

def setup_inputs():
    _rng = _Rng(jax.random.key(int.from_bytes(__import__("os").urandom(4), "little")))
    _w = (lambda a: (lambda t: t.astype(jnp.bfloat16) if jnp.issubdtype(t.dtype, jnp.floating) else t)(jnp.asarray(a)))
    def _A_setup():
        B, Sq, D = 2, 1, 512
        H, Sk, Dh = 32, 8192, 128
        return {
            "x": _w((lambda *s: _rng.normal(s) * 0.05)(B, Sq, D)),
            "k_cache": _w((lambda *s: _rng.normal(s) * 0.05)(B, H, Sk, Dh)),
            "v_cache": _w((lambda *s: _rng.normal(s) * 0.05)(B, H, Sk, Dh)),
            "wq": _w((lambda *s: _rng.normal(s) * 0.05)(D, H * Dh) * (D ** -0.5)),
            "wo": _w((lambda *s: _rng.normal(s) * 0.05)(H * Dh, D) * ((H * Dh) ** -0.5)),
        }
    _A_in = _A_setup()

    def _B_setup():
        B, H, Sq, Sk, D, M = 2, 32, 1, 8192, 128, 512
        Dc = 4 * D
        return {
            "x": _w((lambda *s: _rng.normal(s) * 0.05)(B, Sq, M)),
            "c_kv": _w((lambda *s: _rng.normal(s) * 0.05)(B, Sk, Dc)),
            "w_q": _w((lambda *s: _rng.normal(s) * 0.05)(M, H, D) * (M ** -0.5)),
            "w_uk": _w((lambda *s: _rng.normal(s) * 0.05)(Dc, H, D) * (Dc ** -0.5)),
            "w_uv": _w((lambda *s: _rng.normal(s) * 0.05)(Dc, H, D) * (Dc ** -0.5)),
            "w_o": _w((lambda *s: _rng.normal(s) * 0.05)(H, D, M) * ((H * D) ** -0.5)),
        }
    _B_in = _B_setup()

    return {
        "A_x": _A_in["x"],
        "A_k_cache": _A_in["k_cache"],
        "A_v_cache": _A_in["v_cache"],
        "A_wq": _A_in["wq"],
        "A_wo": _A_in["wo"],
        "B_x": _B_in["x"],
        "B_c_kv": _B_in["c_kv"],
        "B_w_q": _B_in["w_q"],
        "B_w_uk": _B_in["w_uk"],
        "B_w_uv": _B_in["w_uv"],
        "B_w_o": _B_in["w_o"],
        "gate_w": _w((lambda *s: _rng.normal(s) * 0.05)(512)),
    }

def reference(A_x, A_k_cache, A_v_cache, A_wq, A_wo, B_x, B_c_kv, B_w_q, B_w_uk, B_w_uv, B_w_o, gate_w):
    def _A_ref(x, k_cache, v_cache, wq, wo):
        B, Sq, D = x.shape
        H, Dh = 32, 128
        q = (lambda x, *d: x.transpose(*d))((x @ wq).reshape(B, Sq, H, Dh), 0, 2, 1, 3)
        scores = jnp.einsum("bhqd,bhkd->bhqk", q, k_cache) * (Dh ** -0.5)
        p = _softmax(scores, axis=-1)
        o = jnp.einsum("bhqk,bhkd->bhqd", p, v_cache)
        return (lambda x, *d: x.transpose(*d))(o, 0, 2, 1, 3).reshape(B, Sq, H * Dh) @ wo

    def _B_ref(x, c_kv, w_q, w_uk, w_uv, w_o):
        B, Sq, M = x.shape[0], x.shape[1], x.shape[2]
        Sk = c_kv.shape[1]
        H, D = w_q.shape[1], w_q.shape[2]
        q = jnp.einsum("bqm,mhd->bhqd", x, w_q)
        k = jnp.einsum("bkc,chd->bhkd", c_kv, w_uk)
        v = jnp.einsum("bkc,chd->bhkd", c_kv, w_uv)
        scores = jnp.einsum("bhqd,bhkd->bhqk", q, k) * (D ** -0.5)
        off = Sk - Sq
        qi = jnp.arange(Sq)[:, None]
        kj = jnp.arange(Sk)[None, :]
        cmask = kj <= (qi + off)
        scores = jnp.where(cmask[None, None], scores, -1e9)
        p = _softmax(scores, axis=-1)
        ctx = jnp.einsum("bhqk,bhkd->bhqd", p, v)
        return jnp.einsum("bhqd,hdm->bqm", ctx, w_o)

    x = A_x
    g = _sigmoid((x * gate_w).sum(-1, keepdims=True))
    a = _A_ref(x, A_k_cache, A_v_cache, A_wq, A_wo)
    b = _B_ref(x, B_c_kv, B_w_q, B_w_uk, B_w_uv, B_w_o)
    return g * a + (1 - g) * b
```

```python
import jax
import jax.numpy as jnp
from jax import lax
import jax.experimental.pallas as pl
import jax.experimental.pallas.tpu as pltpu

_NT = (((1,), (1,)), ((), ()))
_F32 = jnp.float32
_BF16 = jnp.bfloat16

_NSLOT = 6


def _dot(a, b):
    return jnp.dot(a, b, preferred_element_type=_F32)


def _dot_nt(a, b):
    return lax.dot_general(a, b, _NT, preferred_element_type=_F32)


def _iota(shape, dim):
    return lax.broadcasted_iota(jnp.int32, shape, dim)


def _kernel(
    x_hbm, gate_hbm,
    k_hbm, v_hbm, wq_hbm, wo_hbm, ckv_hbm,
    bwq_hbm, bwuk_hbm, bwuv_hbm, bwo_hbm,
    out_hbm,
    x_ref, gate_ref, out_ref,
    kbuf, vbuf, wq_v, wo_v, ckv_v, bwq_v, bwuk_v, bwuv_v, bwo_v,
    ebig, qa_ref, kv_sems, w_sems,
):
    NR, S, DH = k_hbm.shape
    NB = ckv_hbm.shape[0]
    H = NR // NB
    DM = x_ref.shape[-1]
    DC = ckv_hbm.shape[-1]
    HD = H * DH
    scale = DH ** -0.5

    def k_copy(r, slot):
        return pltpu.make_async_copy(k_hbm.at[r], kbuf.at[slot], kv_sems.at[0, slot])

    def v_copy(r, slot):
        return pltpu.make_async_copy(v_hbm.at[r], vbuf.at[slot], kv_sems.at[1, slot])

    wq_cp = pltpu.make_async_copy(wq_hbm, wq_v, w_sems.at[0])
    bwq_cp = pltpu.make_async_copy(bwq_hbm, bwq_v, w_sems.at[1])
    bwuk_cp = pltpu.make_async_copy(bwuk_hbm, bwuk_v, w_sems.at[2])
    ckv_cp = [pltpu.make_async_copy(ckv_hbm.at[b], ckv_v.at[b], w_sems.at[3 + b])
              for b in range(NB)]
    bwuv_cp = pltpu.make_async_copy(bwuv_hbm, bwuv_v, w_sems.at[3 + NB])
    bwo_cp = pltpu.make_async_copy(bwo_hbm, bwo_v, w_sems.at[4 + NB])
    wo_cp = pltpu.make_async_copy(wo_hbm, wo_v, w_sems.at[5 + NB])

    x_cp = pltpu.make_async_copy(x_hbm, x_ref, w_sems.at[6 + NB])
    gate_cp = pltpu.make_async_copy(gate_hbm, gate_ref, w_sems.at[7 + NB])
    out_cp = pltpu.make_async_copy(out_ref, out_hbm, w_sems.at[8 + NB])
    x_cp.start()
    gate_cp.start()
    bwq_cp.start()
    wq_cp.start()
    bwuk_cp.start()
    for cp in ckv_cp:
        cp.start()
    bwuv_cp.start()
    bwo_cp.start()
    k_copy(0, 0).start()
    v_copy(0, 0).start()
    wo_cp.start()
    for i in range(1, _NSLOT):
        k_copy(i, i).start()
        v_copy(i, i).start()

    ebig[...] = ((_iota((DH, HD), 1) // H) == _iota((DH, HD), 0)).astype(_BF16)
    diag128 = ((_iota((NR, DH), 1) % H) == (_iota((NR, DH), 0) % H)).astype(_F32)
    diag = jnp.tile(diag128, (1, HD // DH))
    row_h = _iota((NR, DH), 0) % H

    def heads_to_rows(a, w_ref):
        acc = None
        for j in range(a.shape[1] // DH):
            aexp = _dot(a[:, j * DH:(j + 1) * DH], ebig[...])
            lhs = (aexp * diag).astype(_BF16)
            part = _dot(lhs, w_ref[j * HD:(j + 1) * HD, :])
            acc = part if acc is None else acc + part
        return acc

    x_cp.wait()
    gate_cp.wait()
    xv = x_ref[...]
    x_rows = [jnp.broadcast_to(xv[b:b + 1, :], (H, DM)) for b in range(NB)]
    xr = jnp.concatenate(x_rows, axis=0)

    bwq_cp.wait()
    qb = heads_to_rows(xr, bwq_v).astype(_BF16)

    wq_cp.wait()
    t = _dot(xr, wq_v[...])
    qa = jnp.zeros((NR, DH), _F32)
    for u in range(H):
        qa = jnp.where(row_h == u, t[:, u * DH:(u + 1) * DH], qa)
    qa_ref[...] = qa.astype(_BF16).astype(_F32)

    bwuk_cp.wait()
    y_parts = []
    for j in range(DC // DH):
        tt = _dot_nt(qb, bwuk_v[j * HD:(j + 1) * HD, :])
        tm = (tt * diag).astype(_BF16)
        y_parts.append(_dot_nt(tm, ebig[...]))
    y = jnp.concatenate(y_parts, axis=1).astype(_BF16)

    ctx = []
    for b in range(NB):
        ckv_cp[b].wait()
        s = _dot_nt(y[b * H:(b + 1) * H, :], ckv_v[b]) * scale
        m = jnp.max(s, axis=-1, keepdims=True)
        p = jnp.exp(s - m)
        l = jnp.sum(p, axis=-1, keepdims=True)
        ctx.append(_dot(p.astype(_BF16), ckv_v[b]) / l)
    ctx = jnp.concatenate(ctx, axis=0).astype(_BF16)

    bwuv_cp.wait()
    ctx_d = heads_to_rows(ctx, bwuv_v)

    bwo_cp.wait()
    lz = jnp.concatenate(
        [jnp.where(row_h == u, ctx_d, 0.0) for u in range(H)], axis=1).astype(_BF16)
    zb = _dot(lz, bwo_v[...])
    row8 = _iota((8, DM), 0)
    out_b = jnp.zeros((8, DM), _F32)
    x8 = jnp.zeros((8, DM), _F32)
    for b in range(NB):
        sb = jnp.sum(zb[b * H:(b + 1) * H, :], axis=0, keepdims=True)
        out_b = jnp.where(row8 == b, sb, out_b)
        x8 = jnp.where(row8 == b, xv[b:b + 1, :].astype(_F32), x8)
    gate = jax.nn.sigmoid(
        jnp.sum(x8 * gate_ref[...].astype(_F32).reshape(1, DM), axis=-1, keepdims=True))

    wo_cp.wait()
    row8d = _iota((8, DH), 0)

    def body(r, acc):
        slot = r % _NSLOT
        b = r // H
        h = r % H
        q = jnp.broadcast_to(qa_ref[pl.ds(r, 1), :], (8, DH)).astype(_BF16)
        k_copy(r, slot).wait()
        s = _dot_nt(q, kbuf[slot]) * scale
        m = jnp.max(s, axis=-1, keepdims=True)
        p = jnp.exp(s - m)
        l = jnp.sum(p, axis=-1, keepdims=True)
        v_copy(r, slot).wait()
        o = _dot(p.astype(_BF16), vbuf[slot]) / l

        @pl.when(r + _NSLOT < NR)
        def _():
            k_copy(r + _NSLOT, slot).start()
            v_copy(r + _NSLOT, slot).start()

        ob = jnp.where(row8d == b, o, 0.0).astype(_BF16)
        w = wo_v[pl.ds(pl.multiple_of(h * DH, DH), DH), :]
        return acc + _dot(ob, w)

    out_a = lax.fori_loop(0, NR, body, jnp.zeros((8, DM), _F32))

    res = (gate * out_a + (1.0 - gate) * out_b).astype(out_ref.dtype)
    out_ref[...] = res[0:NB, :]
    out_cp.start()
    out_cp.wait()


@jax.jit
def pallas_gated_mix__mha_block_cached__compressed_kv_cla__decode_kernel(
    A_x: jax.Array,
    A_k_cache: jax.Array,
    A_v_cache: jax.Array,
    A_wq: jax.Array,
    A_wo: jax.Array,
    B_x: jax.Array,
    B_c_kv: jax.Array,
    B_w_q: jax.Array,
    B_w_uk: jax.Array,
    B_w_uv: jax.Array,
    B_w_o: jax.Array,
    gate_w: jax.Array,
):
    del B_x
    B, H, S, DH = A_k_cache.shape
    DM = A_x.shape[-1]
    DC = B_c_kv.shape[-1]
    NR = B * H

    k = A_k_cache.reshape(NR, S, DH)
    v = A_v_cache.reshape(NR, S, DH)
    bwq = B_w_q.reshape(DM * H, DH)
    bwuk = B_w_uk.reshape(DC * H, DH)
    bwuv = B_w_uv.reshape(DC * H, DH)
    bwo = B_w_o.reshape(H * DH, DM)

    hbm = pl.BlockSpec(memory_space=pl.ANY)
    dt = A_k_cache.dtype

    out = pl.pallas_call(
        _kernel,
        out_shape=jax.ShapeDtypeStruct((B, DM), A_x.dtype),
        in_specs=[hbm] * 11,
        out_specs=hbm,
        scratch_shapes=[
            pltpu.VMEM((B, DM), A_x.dtype),
            pltpu.VMEM(gate_w.shape, gate_w.dtype),
            pltpu.VMEM((B, DM), A_x.dtype),
            pltpu.VMEM((_NSLOT, S, DH), dt),
            pltpu.VMEM((_NSLOT, S, DH), dt),
            pltpu.VMEM(A_wq.shape, dt),
            pltpu.VMEM(A_wo.shape, dt),
            pltpu.VMEM(B_c_kv.shape, dt),
            pltpu.VMEM(bwq.shape, dt),
            pltpu.VMEM(bwuk.shape, dt),
            pltpu.VMEM(bwuv.shape, dt),
            pltpu.VMEM(bwo.shape, dt),
            pltpu.VMEM((DH, H * DH), _BF16),
            pltpu.VMEM((NR, DH), _F32),
            pltpu.SemaphoreType.DMA((2, _NSLOT)),
            pltpu.SemaphoreType.DMA((9 + B,)),
        ],
        compiler_params=pltpu.CompilerParams(vmem_limit_bytes=120 * 1024 * 1024),
    )(A_x.reshape(B, DM), gate_w, k, v, A_wq, A_wo, B_c_kv, bwq, bwuk, bwuv, bwo)
    return out.reshape(B, 1, DM)
```

```python
import jax
import jax.numpy as jnp
from jax import lax
import jax.experimental.pallas as pl
import jax.experimental.pallas.tpu as pltpu

_NT = (((1,), (1,)), ((), ()))
_F32 = jnp.float32
_BF16 = jnp.bfloat16

_CHUNK_BYTES = 32 * 1024
_GH = 8
_NSLOT = 3


def _dot(a, b):
    return jnp.dot(a, b, preferred_element_type=_F32)


def _dot_nt(a, b):
    return lax.dot_general(a, b, _NT, preferred_element_type=_F32)


def _iota(shape, dim):
    return lax.broadcasted_iota(jnp.int32, shape, dim)


def _ds(start, size):
    return pl.ds(pl.multiple_of(start, size), size)


def _kernel(
    x_hbm, gate_hbm, k_hbm, v_hbm, wq_hbm, wo_hbm, ckv_hbm,
    bwq_hbm, bwuk_hbm, bwuv_hbm, bwo_hbm,
    out_hbm,
    x_ref, gate_ref, out_ref, ring,
    wq_v, wo_v, ckv_v, bwq_v, bwuk_v, bwuv_v, bwo_v,
    ebig, qa_ref, qb_ref, y_ref, sb_ref, gmix_ref, bmix_ref,
    s_buf, m_ref, l_ref, acc_ref, outa_ref,
    ring_sems, w_sems,
):
    NR, S, DH = k_hbm.shape
    NB = ckv_hbm.shape[0]
    H = NR // NB
    DM = x_ref.shape[-1]
    DC = ckv_hbm.shape[-1]
    HD = H * DH
    scale = DH ** -0.5

    GH = _GH
    NG = NR // GH
    KB = ring.shape[2]
    NBATCH = S // KB
    CR = _CHUNK_BYTES // (2 * DH)
    L = _NSLOT

    def b_streams(name):
        if name in ("bwq", "bwuk", "bwuv"):
            src, dst, sem = {"bwq": (bwq_hbm, bwq_v, 0), "bwuk": (bwuk_hbm, bwuk_v, 1),
                             "bwuv": (bwuv_hbm, bwuv_v, 2)}[name]
            rows = src.shape[0] // 4

            def mk(s):
                def cp(j):
                    sl = _ds(s * rows + j * CR, CR)
                    return pltpu.make_async_copy(src.at[sl], dst.at[sl], w_sems.at[sem])
                return cp
            return [mk(s) for s in range(4)]
        if name == "wq":
            rows, cols = 16, _CHUNK_BYTES // (2 * 16)
            ncb = wq_hbm.shape[1] // cols
            srows = wq_hbm.shape[0] // 4

            def mk(s):
                def cp(j):
                    idx = (_ds(s * srows + (j // ncb) * rows, rows), _ds((j % ncb) * cols, cols))
                    return pltpu.make_async_copy(wq_hbm.at[idx], wq_v.at[idx], w_sems.at[3])
                return cp
            return [mk(s) for s in range(4)]
        if name in ("wo", "bwo") or name.startswith("ckv"):
            if name == "wo":
                src, dst, sem = wo_hbm, wo_v, 4
            elif name == "bwo":
                src, dst, sem = bwo_hbm, bwo_v, 5
            else:
                b = int(name[3:])
                src, dst, sem = ckv_hbm.at[b], ckv_v.at[b], 6 + b
            cr = _CHUNK_BYTES // (2 * src.shape[1])
            srows = 32 * cr
            ns = src.shape[0] // srows

            def mk(s):
                def cp(j):
                    sl = _ds(s * srows + j * cr, cr)
                    return pltpu.make_async_copy(src.at[sl], dst.at[sl], w_sems.at[sem])
                return cp
            return [mk(s) for s in range(ns)]
        raise ValueError(name)

    def issue_b(streams, j0, j1):
        def body(j, c):
            for i, cp in enumerate(streams):
                cp(j).start(priority=i % 2)
            return c
        lax.fori_loop(j0, j1, body, 0)

    def wait_all(ref, sem):
        pltpu.make_async_copy(ref, ref, w_sems.at[sem]).wait()

    def issue_kv(src, g, b, slot):
        for j in range(KB // CR):
            for hh in range(GH):
                pltpu.make_async_copy(
                    src.at[g * GH + hh, _ds(b * KB + j * CR, CR)],
                    ring.at[slot, hh, pl.ds(j * CR, CR)],
                    ring_sems.at[slot],
                ).start(priority=hh % 2)

    def wait_kv(slot):
        pltpu.make_async_copy(ring.at[slot], ring.at[slot], ring_sems.at[slot]).wait()

    x_cp = pltpu.make_async_copy(x_hbm, x_ref, w_sems.at[6 + NB])
    gate_cp = pltpu.make_async_copy(gate_hbm, gate_ref, w_sems.at[7 + NB])
    out_cp = pltpu.make_async_copy(out_ref, out_hbm, w_sems.at[8 + NB])

    diag128 = ((_iota((NR, DH), 1) % H) == (_iota((NR, DH), 0) % H)).astype(_F32)
    diag = jnp.tile(diag128, (1, HD // DH))
    row_h = _iota((NR, DH), 0) % H

    def x_rows():
        xv = x_ref[...]
        return jnp.concatenate(
            [jnp.broadcast_to(xv[b:b + 1, :], (H, DM)) for b in range(NB)], axis=0)

    def heads_to_rows(a, w_ref, js):
        acc = None
        for j in js:
            aexp = _dot(a[:, j * DH:(j + 1) * DH], ebig[...])
            lhs = (aexp * diag).astype(_BF16)
            part = _dot(lhs, w_ref[j * HD:(j + 1) * HD, :])
            acc = part if acc is None else acc + part
        return acc

    def p_const():
        ebig[...] = ((_iota((DH, HD), 1) // H) == _iota((DH, HD), 0)).astype(_BF16)
        x_cp.wait()
        gate_cp.wait()

    NJ = DM // DH

    def p_bq(half):
        def run():
            if half == 0:
                wait_all(bwq_v, 0)
            js = range(half * (NJ // 2), (half + 1) * (NJ // 2))
            part = heads_to_rows(x_rows(), bwq_v, js)
            if half == 0:
                qb_ref[...] = part
            else:
                qb_ref[...] = qb_ref[...] + part
        return run

    def p_aq():
        wait_all(wq_v, 3)
        t = _dot(x_rows(), wq_v[...])
        qa = jnp.zeros((NR, DH), _F32)
        for u in range(H):
            qa = jnp.where(row_h == u, t[:, u * DH:(u + 1) * DH], qa)
        qa_ref[...] = qa.astype(_BF16).astype(_F32)

    def p_by(half):
        def run():
            if half == 0:
                wait_all(bwuk_v, 1)
            qb = qb_ref[...].astype(_BF16)
            nj = DC // DH
            for j in range(half * (nj // 2), (half + 1) * (nj // 2)):
                tt = _dot_nt(qb, bwuk_v[j * HD:(j + 1) * HD, :])
                tm = (tt * diag).astype(_BF16)
                y_ref[:, j * DH:(j + 1) * DH] = _dot_nt(tm, ebig[...])
        return run

    def p_scores(b, half):
        def run():
            if half == 0:
                wait_all(ckv_v.at[b], 6 + b)
            yb = y_ref[b * H:(b + 1) * H, :].astype(_BF16)
            ks = slice(half * (S // 2), (half + 1) * (S // 2))
            sb_ref[:, ks] = _dot_nt(yb, ckv_v[b, ks, :]) * scale
        return run

    def p_softmax(b):
        def run():
            s = sb_ref[...]
            m = jnp.max(s, axis=-1, keepdims=True)
            p = jnp.exp(s - m)
            sb_ref[...] = p / jnp.sum(p, axis=-1, keepdims=True)
        return run

    def p_ctx(b):
        def run():
            y_ref[b * H:(b + 1) * H, :] = _dot(sb_ref[...].astype(_BF16), ckv_v[b])
        return run

    def p_buv(half):
        def run():
            if half == 0:
                wait_all(bwuv_v, 2)
            nj = DC // DH
            js = range(half * (nj // 2), (half + 1) * (nj // 2))
            part = heads_to_rows(y_ref[...].astype(_BF16), bwuv_v, js)
            if half == 0:
                qb_ref[...] = part
            else:
                qb_ref[...] = qb_ref[...] + part
        return run

    def p_bo():
        wait_all(bwo_v, 5)
        ctx_d = qb_ref[...].astype(_BF16).astype(_F32)
        lz = jnp.concatenate(
            [jnp.where(row_h == u, ctx_d, 0.0) for u in range(H)], axis=1).astype(_BF16)
        zb = _dot(lz, bwo_v[...])
        row8 = _iota((8, DM), 0)
        xv = x_ref[...].astype(_F32)
        out_b = jnp.zeros((8, DM), _F32)
        x8 = jnp.zeros((8, DM), _F32)
        for b in range(NB):
            sb = jnp.sum(zb[b * H:(b + 1) * H, :], axis=0, keepdims=True)
            out_b = jnp.where(row8 == b, sb, out_b)
            x8 = jnp.where(row8 == b, xv[b:b + 1, :], x8)
        gate = jax.nn.sigmoid(jnp.sum(
            x8 * gate_ref[...].astype(_F32).reshape(1, DM), axis=-1, keepdims=True))
        gmix_ref[...] = jnp.broadcast_to(gate, (8, DM))
        bmix_ref[...] = (1.0 - gate) * out_b
        outa_ref[...] = jnp.zeros((8, DM), _F32)

    def p_wo():
        wait_all(wo_v, 4)

    def idle():
        pass

    NLT = KB // DH

    def fold(a):
        return [a[:, t * DH:(t + 1) * DH] for t in range(NLT)]

    def k_unit(g, b, slot):
        for hh in range(GH):
            q = jnp.broadcast_to(qa_ref[pl.ds(g * GH + hh, 1), :], (8, DH)).astype(_BF16)
            s = _dot_nt(q, ring[slot, hh]) * scale
            s_buf[hh, b] = s
            m = m_ref[hh]
            for t in fold(s):
                m = jnp.maximum(m, t)
            m_ref[hh] = m

    def v_unit(b, slot):
        for hh in range(GH):
            p = jnp.exp(s_buf[hh, b] - jnp.tile(m_ref[hh], (1, NLT)))
            l = l_ref[hh]
            for t in fold(p):
                l = l + t
            l_ref[hh] = l
            acc_ref[hh] = acc_ref[hh] + _dot(p.astype(_BF16), ring[slot, hh])

    def k_begin():
        m_ref[...] = jnp.full(m_ref.shape, -jnp.inf, _F32)

    def v_begin():
        for hh in range(GH):
            m = jnp.max(m_ref[hh], axis=-1, keepdims=True)
            m_ref[hh] = jnp.broadcast_to(m, (8, DH))
        l_ref[...] = jnp.zeros(l_ref.shape, _F32)
        acc_ref[...] = jnp.zeros(acc_ref.shape, _F32)

    def group_end(g):
        row8d = _iota((8, DH), 0)
        bidx = (g * GH) // H
        h0 = (g * GH) % H
        out = outa_ref[...]
        for hh in range(GH):
            l = jnp.sum(l_ref[hh], axis=-1, keepdims=True)
            o = jnp.where(row8d == bidx, acc_ref[hh] / l, 0.0).astype(_BF16)
            out = out + _dot(o, wo_v[_ds((h0 + hh) * DH, DH), :])
        outa_ref[...] = out

    x_cp.start()
    gate_cp.start()
    s1 = b_streams("bwq") + b_streams("wq")
    s2 = b_streams("bwuk") + b_streams("wo")
    s3 = b_streams("ckv0")
    s4 = b_streams("ckv1")
    s5 = b_streams("bwuv") + b_streams("bwo")
    stages = [
        (s1, [p_const, idle, idle, idle]),
        (s2, [p_bq(0), p_bq(1), p_aq, idle]),
        (s3, [p_by(0), p_by(1), idle, idle]),
        (s4, [p_scores(0, 0), p_scores(0, 1), p_softmax(0), p_ctx(0)]),
        (s5, [p_scores(1, 0), p_scores(1, 1), p_softmax(1), p_ctx(1)]),
    ]
    for streams, pieces in stages:
        for i, piece in enumerate(pieces):
            issue_b(streams, 8 * i, 8 * (i + 1))
            piece()

    tail_pieces = [p_buv(0), p_buv(1), p_bo]
    for u in range(L):
        issue_kv(k_hbm, 0, u, u % L)
        if u < len(tail_pieces):
            tail_pieces[u]()
    for piece in tail_pieces[L:]:
        piece()
    p_wo()

    def group_body(g, c):
        base = g * (2 * NBATCH)

        def slot_of(u):
            return (base + u) % L

        k_begin()

        def k_same(b, c):
            wait_kv(slot_of(b))
            k_unit(g, b, slot_of(b))
            issue_kv(k_hbm, g, b + L, slot_of(b))
            return c
        lax.fori_loop(0, NBATCH - L, k_same, 0)

        def k_next(b, c):
            wait_kv(slot_of(b))
            k_unit(g, b, slot_of(b))
            issue_kv(v_hbm, g, b + L - NBATCH, slot_of(b))
            return c
        lax.fori_loop(NBATCH - L, NBATCH, k_next, 0)

        v_begin()

        def v_same(b, c):
            wait_kv(slot_of(NBATCH + b))
            v_unit(b, slot_of(NBATCH + b))
            issue_kv(v_hbm, g, b + L, slot_of(NBATCH + b))
            return c
        lax.fori_loop(0, NBATCH - L, v_same, 0)

        def v_next(b, c):
            wait_kv(slot_of(NBATCH + b))
            v_unit(b, slot_of(NBATCH + b))

            @pl.when(g + 1 < NG)
            def _():
                issue_kv(k_hbm, g + 1, b + L - NBATCH, slot_of(NBATCH + b))
            return c
        lax.fori_loop(NBATCH - L, NBATCH, v_next, 0)

        group_end(g)
        return c

    lax.fori_loop(0, NG, group_body, 0)

    res = gmix_ref[...] * outa_ref[...] + bmix_ref[...]
    out_ref[...] = res[0:NB, :].astype(out_ref.dtype)
    out_cp.start()
    out_cp.wait()


@jax.jit
def pallas_gated_mix__mha_block_cached__compressed_kv_cla__decode_kernel(
    A_x: jax.Array,
    A_k_cache: jax.Array,
    A_v_cache: jax.Array,
    A_wq: jax.Array,
    A_wo: jax.Array,
    B_x: jax.Array,
    B_c_kv: jax.Array,
    B_w_q: jax.Array,
    B_w_uk: jax.Array,
    B_w_uv: jax.Array,
    B_w_o: jax.Array,
    gate_w: jax.Array,
):
    del B_x
    B, H, S, DH = A_k_cache.shape
    DM = A_x.shape[-1]
    DC = B_c_kv.shape[-1]
    NR = B * H
    KB = (64 * _CHUNK_BYTES) // (_GH * DH * 2)

    k = A_k_cache.reshape(NR, S, DH)
    v = A_v_cache.reshape(NR, S, DH)
    bwq = B_w_q.reshape(DM * H, DH)
    bwuk = B_w_uk.reshape(DC * H, DH)
    bwuv = B_w_uv.reshape(DC * H, DH)
    bwo = B_w_o.reshape(H * DH, DM)

    hbm = pl.BlockSpec(memory_space=pl.ANY)
    dt = A_k_cache.dtype

    out = pl.pallas_call(
        _kernel,
        out_shape=jax.ShapeDtypeStruct((B, DM), A_x.dtype),
        in_specs=[hbm] * 11,
        out_specs=hbm,
        scratch_shapes=[
            pltpu.VMEM((B, DM), A_x.dtype),
            pltpu.VMEM(gate_w.shape, gate_w.dtype),
            pltpu.VMEM((B, DM), A_x.dtype),
            pltpu.VMEM((_NSLOT, _GH, KB, DH), dt),
            pltpu.VMEM(A_wq.shape, dt),
            pltpu.VMEM(A_wo.shape, dt),
            pltpu.VMEM(B_c_kv.shape, dt),
            pltpu.VMEM(bwq.shape, dt),
            pltpu.VMEM(bwuk.shape, dt),
            pltpu.VMEM(bwuv.shape, dt),
            pltpu.VMEM(bwo.shape, dt),
            pltpu.VMEM((DH, H * DH), _BF16),
            pltpu.VMEM((NR, DH), _F32),
            pltpu.VMEM((NR, DH), _F32),
            pltpu.VMEM((NR, DC), _F32),
            pltpu.VMEM((H, S), _F32),
            pltpu.VMEM((8, DM), _F32),
            pltpu.VMEM((8, DM), _F32),
            pltpu.VMEM((_GH, S // KB, 8, KB), _F32),
            pltpu.VMEM((_GH, 8, DH), _F32),
            pltpu.VMEM((_GH, 8, DH), _F32),
            pltpu.VMEM((_GH, 8, DH), _F32),
            pltpu.VMEM((8, DM), _F32),
            pltpu.SemaphoreType.DMA((_NSLOT,)),
            pltpu.SemaphoreType.DMA((9 + B,)),
        ],
        compiler_params=pltpu.CompilerParams(vmem_limit_bytes=100 * 1024 * 1024),
    )(A_x.reshape(B, DM), gate_w, k, v, A_wq, A_wo, B_c_kv, bwq, bwuk, bwuv, bwo)
    return out.reshape(B, 1, DM)
```

```python
import jax
import jax.numpy as jnp
from jax import lax
import jax.experimental.pallas as pl
import jax.experimental.pallas.tpu as pltpu

_NT = (((1,), (1,)), ((), ()))
_F32 = jnp.float32
_BF16 = jnp.bfloat16

_CHUNK_BYTES = 32 * 1024
_NDESC = 64
_GH = 16
_NSLOT = 3
_PAIR = 2
_HOIST = True


def _dot(a, b):
    return jnp.dot(a, b, preferred_element_type=_F32)


def _dot_nt(a, b):
    return lax.dot_general(a, b, _NT, preferred_element_type=_F32)


def _iota(shape, dim):
    return lax.broadcasted_iota(jnp.int32, shape, dim)


def _ds(start, size):
    return pl.ds(pl.multiple_of(start, size), size)


def _kernel(
    x_hbm, gate_hbm, k_hbm, v_hbm, wq_hbm, wo_hbm, ckv_hbm,
    bwq_hbm, bwuk_hbm, bwuv_hbm, bwo_hbm,
    out_hbm,
    x_ref, gate_ref, out_ref, ring,
    wq_v, wo_v, ckv_v, bwq_v, bwuk_v, bwuv_v, bwo_v,
    ebig, qa_ref, qb_ref, y_ref, sb_ref, gmix_ref, bmix_ref,
    s_buf, m_ref, l_ref, acc_ref, outa_ref,
    ring_sems, w_sems,
):
    NR, S, DH = k_hbm.shape
    NB = ckv_hbm.shape[0]
    H = NR // NB
    DM = x_ref.shape[-1]
    DC = ckv_hbm.shape[-1]
    HD = H * DH
    scale = DH ** -0.5

    GH = _GH
    NG = NR // GH
    KB = ring.shape[2]
    NBATCH = S // KB
    CR = _CHUNK_BYTES // (2 * DH)
    L = _NSLOT
    SCH = (1024 * 1024) // _CHUNK_BYTES

    def b_streams(name):
        if name in ("bwq", "bwuk", "bwuv"):
            src, dst, sem = {"bwq": (bwq_hbm, bwq_v, 0), "bwuk": (bwuk_hbm, bwuk_v, 1),
                             "bwuv": (bwuv_hbm, bwuv_v, 2)}[name]
            rows = SCH * CR

            def mk(s):
                def cp(j):
                    sl = _ds(s * rows + j * CR, CR)
                    return pltpu.make_async_copy(src.at[sl], dst.at[sl], w_sems.at[sem])
                return cp
            return [mk(s) for s in range(src.shape[0] // rows)]
        if name == "wq":
            rows, cols = 16, _CHUNK_BYTES // (2 * 16)
            ncb = wq_hbm.shape[1] // cols
            srows = (SCH // ncb) * rows

            def mk(s):
                def cp(j):
                    idx = (_ds(s * srows + (j // ncb) * rows, rows), _ds((j % ncb) * cols, cols))
                    return pltpu.make_async_copy(wq_hbm.at[idx], wq_v.at[idx], w_sems.at[3])
                return cp
            return [mk(s) for s in range(wq_hbm.shape[0] // srows)]
        if name in ("wo", "bwo") or name.startswith("ckv"):
            if name == "wo":
                src, dst, sem = wo_hbm, wo_v, 4
            elif name == "bwo":
                src, dst, sem = bwo_hbm, bwo_v, 5
            else:
                b = int(name[3:])
                src, dst, sem = ckv_hbm.at[b], ckv_v.at[b], 6 + b
            cr = _CHUNK_BYTES // (2 * src.shape[1])
            srows = SCH * cr
            ns = src.shape[0] // srows

            def mk(s):
                def cp(j):
                    sl = _ds(s * srows + j * cr, cr)
                    return pltpu.make_async_copy(src.at[sl], dst.at[sl], w_sems.at[sem])
                return cp
            return [mk(s) for s in range(ns)]
        raise ValueError(name)

    def b_batches(*names):
        streams = [cp for name in names for cp in b_streams(name)]
        jb = _NDESC // len(streams)

        def mk(j0):
            def run():
                def body(j, c):
                    for i, cp in enumerate(streams):
                        cp(j).start(priority=i % 2)
                    return c
                lax.fori_loop(j0, j0 + jb, body, 0)
            return run
        return [mk(j0) for j0 in range(0, SCH, jb)]

    def wait_all(ref, sem):
        pltpu.make_async_copy(ref, ref, w_sems.at[sem]).wait()

    def issue_kv(src, g, b, slot):
        for j in range(KB // CR):
            for hh in range(GH):
                pltpu.make_async_copy(
                    src.at[g * GH + hh, _ds(b * KB + j * CR, CR)],
                    ring.at[slot, hh, pl.ds(j * CR, CR)],
                    ring_sems.at[slot],
                ).start(priority=hh % 2)

    def wait_kv(slot):
        pltpu.make_async_copy(ring.at[slot], ring.at[slot], ring_sems.at[slot]).wait()

    x_cp = pltpu.make_async_copy(x_hbm, x_ref, w_sems.at[6 + NB])
    gate_cp = pltpu.make_async_copy(gate_hbm, gate_ref, w_sems.at[7 + NB])
    out_cp = pltpu.make_async_copy(out_ref, out_hbm, w_sems.at[8 + NB])

    diag128 = ((_iota((NR, DH), 1) % H) == (_iota((NR, DH), 0) % H)).astype(_F32)
    diag = jnp.tile(diag128, (1, HD // DH))
    row_h = _iota((NR, DH), 0) % H

    def x_rows():
        xv = x_ref[...]
        return jnp.concatenate(
            [jnp.broadcast_to(xv[b:b + 1, :], (H, DM)) for b in range(NB)], axis=0)

    def heads_to_rows(a, w_ref, js):
        acc = None
        for j in js:
            aexp = _dot(a[:, j * DH:(j + 1) * DH], ebig[...])
            lhs = (aexp * diag).astype(_BF16)
            part = _dot(lhs, w_ref[j * HD:(j + 1) * HD, :])
            acc = part if acc is None else acc + part
        return acc

    def p_const():
        ebig[...] = ((_iota((DH, HD), 1) // H) == _iota((DH, HD), 0)).astype(_BF16)
        x_cp.wait()
        gate_cp.wait()

    NJ = DM // DH

    def p_bq(half):
        def run():
            if half == 0:
                wait_all(bwq_v, 0)
            js = range(half * (NJ // 2), (half + 1) * (NJ // 2))
            part = heads_to_rows(x_rows(), bwq_v, js)
            if half == 0:
                qb_ref[...] = part
            else:
                qb_ref[...] = qb_ref[...] + part
        return run

    def p_aq():
        wait_all(wq_v, 3)
        t = _dot(x_rows(), wq_v[...])
        qa = jnp.zeros((NR, DH), _F32)
        for u in range(H):
            qa = jnp.where(row_h == u, t[:, u * DH:(u + 1) * DH], qa)
        qa_ref[...] = qa.astype(_BF16).astype(_F32)

    def p_by(half):
        def run():
            if half == 0:
                wait_all(bwuk_v, 1)
            qb = qb_ref[...].astype(_BF16)
            nj = DC // DH
            for j in range(half * (nj // 2), (half + 1) * (nj // 2)):
                tt = _dot_nt(qb, bwuk_v[j * HD:(j + 1) * HD, :])
                tm = (tt * diag).astype(_BF16)
                y_ref[:, j * DH:(j + 1) * DH] = _dot_nt(tm, ebig[...])
        return run

    def p_scores(b, half):
        def run():
            if half == 0:
                wait_all(ckv_v.at[b], 6 + b)
            yb = y_ref[b * H:(b + 1) * H, :].astype(_BF16)
            ks = slice(half * (S // 2), (half + 1) * (S // 2))
            sb_ref[:, ks] = _dot_nt(yb, ckv_v[b, ks, :]) * scale
        return run

    def p_softmax(b):
        def run():
            s = sb_ref[...]
            m = jnp.max(s, axis=-1, keepdims=True)
            p = jnp.exp(s - m)
            sb_ref[...] = p / jnp.sum(p, axis=-1, keepdims=True)
        return run

    def p_ctx(b):
        def run():
            y_ref[b * H:(b + 1) * H, :] = _dot(sb_ref[...].astype(_BF16), ckv_v[b])
        return run

    def p_buv(half):
        def run():
            if half == 0:
                wait_all(bwuv_v, 2)
            nj = DC // DH
            js = range(half * (nj // 2), (half + 1) * (nj // 2))
            part = heads_to_rows(y_ref[...].astype(_BF16), bwuv_v, js)
            if half == 0:
                qb_ref[...] = part
            else:
                qb_ref[...] = qb_ref[...] + part
        return run

    def p_bo():
        wait_all(bwo_v, 5)
        ctx_d = qb_ref[...].astype(_BF16).astype(_F32)
        lz = jnp.concatenate(
            [jnp.where(row_h == u, ctx_d, 0.0) for u in range(H)], axis=1).astype(_BF16)
        zb = _dot(lz, bwo_v[...])
        row8 = _iota((8, DM), 0)
        out_b = jnp.zeros((8, DM), _F32)
        for b in range(NB):
            sb = jnp.sum(zb[b * H:(b + 1) * H, :], axis=0, keepdims=True)
            out_b = jnp.where(row8 == b, sb, out_b)
        bmix_ref[...] = out_b

    def p_gate():
        row8 = _iota((8, DM), 0)
        xv = x_ref[...].astype(_F32)
        x8 = jnp.zeros((8, DM), _F32)
        for b in range(NB):
            x8 = jnp.where(row8 == b, xv[b:b + 1, :], x8)
        gate = jax.nn.sigmoid(jnp.sum(
            x8 * gate_ref[...].astype(_F32).reshape(1, DM), axis=-1, keepdims=True))
        gmix_ref[...] = jnp.broadcast_to(gate, (8, DM))
        outa_ref[...] = jnp.zeros((8, DM), _F32)

    def p_wo():
        wait_all(wo_v, 4)

    NLT = KB // DH

    def fold(a):
        return [a[:, t * DH:(t + 1) * DH] for t in range(NLT)]

    def k_unit(g, b, slot):
        for hh in range(GH):
            q = jnp.broadcast_to(qa_ref[pl.ds(g * GH + hh, 1), :], (8, DH)).astype(_BF16)
            s = _dot_nt(q, ring[slot, hh]) * scale
            s_buf[hh, b] = s
            m = m_ref[hh]
            for t in fold(s):
                m = jnp.maximum(m, t)
            m_ref[hh] = m

    def v_probs(b):
        ps = []
        for hh in range(GH):
            p = jnp.exp(s_buf[hh, b] - jnp.tile(m_ref[hh], (1, NLT)))
            l = l_ref[hh]
            for t in fold(p):
                l = l + t
            l_ref[hh] = l
            ps.append(p.astype(_BF16))
        return ps

    def v_matmul(ps, slot):
        for hh in range(GH):
            acc_ref[hh] = acc_ref[hh] + _dot(ps[hh], ring[slot, hh])

    def v_unit(b, slot):
        if _HOIST:
            ps = v_probs(b)
            wait_kv(slot)
        else:
            wait_kv(slot)
            ps = v_probs(b)
        v_matmul(ps, slot)

    def k_begin():
        m_ref[...] = jnp.full(m_ref.shape, -jnp.inf, _F32)

    def v_begin():
        for hh in range(GH):
            m = jnp.max(m_ref[hh], axis=-1, keepdims=True)
            m_ref[hh] = jnp.broadcast_to(m, (8, DH))
        l_ref[...] = jnp.zeros(l_ref.shape, _F32)
        acc_ref[...] = jnp.zeros(acc_ref.shape, _F32)

    def group_end(g):
        row8d = _iota((8, DH), 0)
        bidx = (g * GH) // H
        h0 = (g * GH) % H
        out = outa_ref[...]
        for hh in range(GH):
            l = jnp.sum(l_ref[hh], axis=-1, keepdims=True)
            o = jnp.where(row8d == bidx, acc_ref[hh] / l, 0.0).astype(_BF16)
            out = out + _dot(o, wo_v[_ds((h0 + hh) * DH, DH), :])
        outa_ref[...] = out

    x_cp.start()
    gate_cp.start()
    for run in (b_batches("wq", "wo") if _PAIR == 2 else b_batches("wq")):
        run()
    pro = [p_const, p_gate, p_aq]
    for u in range(L):
        issue_kv(k_hbm, 0, u, u % L)
        if u < len(pro):
            pro[u]()
    for piece in pro[L:]:
        piece()

    extras = {}

    def attach(u, *fns):
        extras.setdefault(u, []).extend(fns)

    u = 0
    done_at = {}
    if _PAIR == 1:
        order = (("bwq", "wo"), ("bwuk", "bwuv"), ("ckv0",), ("ckv1",), ("bwo",))
    else:
        order = (("bwq", "bwo"), ("bwuk", "bwuv"), ("ckv0",), ("ckv1",))
        done_at["wo"] = 0
    for names in order:
        for run in b_batches(*names):
            attach(u, run)
            u += 1
        for name in names:
            done_at[name] = u
    n_load_units = u

    def chain(u, pieces):
        for piece in pieces:
            attach(u, piece)
            u += 1
        return u
    u = chain(done_at["bwq"] + 1, [p_bq(0), p_bq(1)])
    u = chain(max(u, done_at["bwuk"] + 1), [p_by(0), p_by(1)])
    u = chain(max(u, done_at["ckv0"] + 1),
              [p_scores(0, 0), p_scores(0, 1), p_softmax(0), p_ctx(0)])
    u = chain(max(u, done_at["ckv1"] + 1),
              [p_scores(1, 0), p_scores(1, 1), p_softmax(1), p_ctx(1)])
    u = chain(max(u, done_at["bwuv"] + 1), [p_buv(0), p_buv(1)])
    u = chain(max(u, done_at["bwo"] + 1), [p_bo])
    assert u <= NG * 2 * NBATCH and n_load_units <= 2 * NBATCH * NG
    assert done_at["wo"] + 1 < 2 * NBATCH
    attach(done_at["wo"] + 1, p_wo)

    def run_extras(phase, lo, hi, g, b):
        for uu in sorted(extras):
            eg, ephase, eb = uu // (2 * NBATCH), (uu // NBATCH) % 2, uu % NBATCH
            if ephase == phase and lo <= eb < hi:
                for fn in extras[uu]:
                    pl.when(jnp.logical_and(g == eg, b == eb))(fn)

    def group_body(g, c):
        base = g * (2 * NBATCH)

        def slot_of(u):
            return (base + u) % L

        k_begin()

        def k_same(b, c):
            wait_kv(slot_of(b))
            k_unit(g, b, slot_of(b))
            issue_kv(k_hbm, g, b + L, slot_of(b))
            run_extras(0, 0, NBATCH - L, g, b)
            return c
        lax.fori_loop(0, NBATCH - L, k_same, 0)

        def k_next(b, c):
            wait_kv(slot_of(b))
            k_unit(g, b, slot_of(b))
            issue_kv(v_hbm, g, b + L - NBATCH, slot_of(b))
            run_extras(0, NBATCH - L, NBATCH, g, b)
            return c
        lax.fori_loop(NBATCH - L, NBATCH, k_next, 0)

        v_begin()

        def v_same(b, c):
            v_unit(b, slot_of(NBATCH + b))
            issue_kv(v_hbm, g, b + L, slot_of(NBATCH + b))
            run_extras(1, 0, NBATCH - L, g, b)
            return c
        lax.fori_loop(0, NBATCH - L, v_same, 0)

        def v_next(b, c):
            v_unit(b, slot_of(NBATCH + b))

            @pl.when(g + 1 < NG)
            def _():
                issue_kv(k_hbm, g + 1, b + L - NBATCH, slot_of(NBATCH + b))
            run_extras(1, NBATCH - L, NBATCH, g, b)
            return c
        lax.fori_loop(NBATCH - L, NBATCH, v_next, 0)

        group_end(g)
        return c

    lax.fori_loop(0, NG, group_body, 0)

    gate = gmix_ref[...]
    res = gate * outa_ref[...] + (1.0 - gate) * bmix_ref[...]
    out_ref[...] = res[0:NB, :].astype(out_ref.dtype)
    out_cp.start()
    out_cp.wait()


@jax.jit
def pallas_gated_mix__mha_block_cached__compressed_kv_cla__decode_kernel(
    A_x: jax.Array,
    A_k_cache: jax.Array,
    A_v_cache: jax.Array,
    A_wq: jax.Array,
    A_wo: jax.Array,
    B_x: jax.Array,
    B_c_kv: jax.Array,
    B_w_q: jax.Array,
    B_w_uk: jax.Array,
    B_w_uv: jax.Array,
    B_w_o: jax.Array,
    gate_w: jax.Array,
):
    del B_x
    B, H, S, DH = A_k_cache.shape
    DM = A_x.shape[-1]
    DC = B_c_kv.shape[-1]
    NR = B * H
    KB = (_NDESC * _CHUNK_BYTES) // (_GH * DH * 2)

    k = A_k_cache.reshape(NR, S, DH)
    v = A_v_cache.reshape(NR, S, DH)
    bwq = B_w_q.reshape(DM * H, DH)
    bwuk = B_w_uk.reshape(DC * H, DH)
    bwuv = B_w_uv.reshape(DC * H, DH)
    bwo = B_w_o.reshape(H * DH, DM)

    hbm = pl.BlockSpec(memory_space=pl.ANY)
    dt = A_k_cache.dtype

    out = pl.pallas_call(
        _kernel,
        out_shape=jax.ShapeDtypeStruct((B, DM), A_x.dtype),
        in_specs=[hbm] * 11,
        out_specs=hbm,
        scratch_shapes=[
            pltpu.VMEM((B, DM), A_x.dtype),
            pltpu.VMEM(gate_w.shape, gate_w.dtype),
            pltpu.VMEM((B, DM), A_x.dtype),
            pltpu.VMEM((_NSLOT, _GH, KB, DH), dt),
            pltpu.VMEM(A_wq.shape, dt),
            pltpu.VMEM(A_wo.shape, dt),
            pltpu.VMEM(B_c_kv.shape, dt),
            pltpu.VMEM(bwq.shape, dt),
            pltpu.VMEM(bwuk.shape, dt),
            pltpu.VMEM(bwuv.shape, dt),
            pltpu.VMEM(bwo.shape, dt),
            pltpu.VMEM((DH, H * DH), _BF16),
            pltpu.VMEM((NR, DH), _F32),
            pltpu.VMEM((NR, DH), _F32),
            pltpu.VMEM((NR, DC), _F32),
            pltpu.VMEM((H, S), _F32),
            pltpu.VMEM((8, DM), _F32),
            pltpu.VMEM((8, DM), _F32),
            pltpu.VMEM((_GH, S // KB, 8, KB), _F32),
            pltpu.VMEM((_GH, 8, DH), _F32),
            pltpu.VMEM((_GH, 8, DH), _F32),
            pltpu.VMEM((_GH, 8, DH), _F32),
            pltpu.VMEM((8, DM), _F32),
            pltpu.SemaphoreType.DMA((_NSLOT,)),
            pltpu.SemaphoreType.DMA((9 + B,)),
        ],
        compiler_params=pltpu.CompilerParams(vmem_limit_bytes=100 * 1024 * 1024),
    )(A_x.reshape(B, DM), gate_w, k, v, A_wq, A_wo, B_c_kv, bwq, bwuk, bwuv, bwo)
    return out.reshape(B, 1, DM)
```

```python
import jax
import jax.numpy as jnp
from jax import lax
import jax.experimental.pallas as pl
import jax.experimental.pallas.tpu as pltpu

_NT = (((1,), (1,)), ((), ()))
_F32 = jnp.float32
_BF16 = jnp.bfloat16

_CHUNK_BYTES = 32 * 1024
_NDESC = 64
_GH = 16
_NSLOT = 3
_BORDER = 1


def _dot(a, b):
    return jnp.dot(a, b, preferred_element_type=_F32)


def _dot_nt(a, b):
    return lax.dot_general(a, b, _NT, preferred_element_type=_F32)


def _iota(shape, dim):
    return lax.broadcasted_iota(jnp.int32, shape, dim)


def _ds(start, size):
    return pl.ds(pl.multiple_of(start, size), size)


def _kernel(
    x_hbm, gate_hbm, k_hbm, v_hbm, wq_hbm, wo_hbm, ckv_hbm,
    bwq_hbm, bwuk_hbm, bwuv_hbm, bwo_hbm,
    out_hbm,
    x_ref, gate_ref, out_ref, ring,
    wq_v, wo_v, ckv_v, bwq_v, bwuk_v, bwuv_v, bwo_v,
    ebig, qa_ref, qb_ref, y_ref, sb_ref, gmix_ref, bmix_ref,
    s_buf, m_ref, l_ref, acc_ref, outa_ref,
    ring_sems, w_sems,
):
    NR, S, DH = k_hbm.shape
    NB = ckv_hbm.shape[0]
    H = NR // NB
    DM = x_ref.shape[-1]
    DC = ckv_hbm.shape[-1]
    HD = H * DH
    scale = DH ** -0.5

    GH = _GH
    NG = NR // GH
    KB = ring.shape[2]
    NBATCH = S // KB
    CR = _CHUNK_BYTES // (2 * DH)
    L = _NSLOT
    SCH = (1024 * 1024) // _CHUNK_BYTES

    def b_streams(name):
        if name in ("bwq", "bwuk", "bwuv"):
            src, dst, sem = {"bwq": (bwq_hbm, bwq_v, 0), "bwuk": (bwuk_hbm, bwuk_v, 1),
                             "bwuv": (bwuv_hbm, bwuv_v, 2)}[name]
            rows = SCH * CR

            def mk(s):
                def cp(j):
                    sl = _ds(s * rows + j * CR, CR)
                    return pltpu.make_async_copy(src.at[sl], dst.at[sl], w_sems.at[sem])
                return cp
            return [mk(s) for s in range(src.shape[0] // rows)]
        if name == "wq":
            rows, cols = 16, _CHUNK_BYTES // (2 * 16)
            ncb = wq_hbm.shape[1] // cols
            srows = (SCH // ncb) * rows

            def mk(s):
                def cp(j):
                    idx = (_ds(s * srows + (j // ncb) * rows, rows), _ds((j % ncb) * cols, cols))
                    return pltpu.make_async_copy(wq_hbm.at[idx], wq_v.at[idx], w_sems.at[3])
                return cp
            return [mk(s) for s in range(wq_hbm.shape[0] // srows)]
        if name in ("wo", "bwo") or name.startswith("ckv"):
            if name == "wo":
                src, dst, sem = wo_hbm, wo_v, 4
            elif name == "bwo":
                src, dst, sem = bwo_hbm, bwo_v, 5
            else:
                b = int(name[3:])
                src, dst, sem = ckv_hbm.at[b], ckv_v.at[b], 6 + b
            cr = _CHUNK_BYTES // (2 * src.shape[1])
            srows = SCH * cr
            ns = src.shape[0] // srows

            def mk(s):
                def cp(j):
                    sl = _ds(s * srows + j * cr, cr)
                    return pltpu.make_async_copy(src.at[sl], dst.at[sl], w_sems.at[sem])
                return cp
            return [mk(s) for s in range(ns)]
        raise ValueError(name)

    def b_batches(*names):
        streams = [cp for name in names for cp in b_streams(name)]
        jb = _NDESC // len(streams)

        def mk(j0):
            def run():
                def body(j, c):
                    for i, cp in enumerate(streams):
                        cp(j).start(priority=i % 2)
                    return c
                lax.fori_loop(j0, j0 + jb, body, 0)
            return run
        return [mk(j0) for j0 in range(0, SCH, jb)]

    def wait_all(ref, sem):
        pltpu.make_async_copy(ref, ref, w_sems.at[sem]).wait()

    def issue_kv(src, g, b, slot):
        for j in range(KB // CR):
            for hh in range(GH):
                pltpu.make_async_copy(
                    src.at[g * GH + hh, _ds(b * KB + j * CR, CR)],
                    ring.at[slot, hh, pl.ds(j * CR, CR)],
                    ring_sems.at[slot],
                ).start(priority=hh % 2)

    def wait_kv(slot):
        pltpu.make_async_copy(ring.at[slot], ring.at[slot], ring_sems.at[slot]).wait()

    x_cp = pltpu.make_async_copy(x_hbm, x_ref, w_sems.at[6 + NB])
    gate_cp = pltpu.make_async_copy(gate_hbm, gate_ref, w_sems.at[7 + NB])
    out_cp = pltpu.make_async_copy(out_ref, out_hbm, w_sems.at[8 + NB])

    diag128 = ((_iota((NR, DH), 1) % H) == (_iota((NR, DH), 0) % H)).astype(_F32)
    diag = jnp.tile(diag128, (1, HD // DH))
    row_h = _iota((NR, DH), 0) % H

    def x_rows():
        xv = x_ref[...]
        return jnp.concatenate(
            [jnp.broadcast_to(xv[b:b + 1, :], (H, DM)) for b in range(NB)], axis=0)

    def heads_to_rows(a, w_ref, js):
        acc = None
        for j in js:
            aexp = _dot(a[:, j * DH:(j + 1) * DH], ebig[...])
            lhs = (aexp * diag).astype(_BF16)
            part = _dot(lhs, w_ref[j * HD:(j + 1) * HD, :])
            acc = part if acc is None else acc + part
        return acc

    def p_const():
        ebig[...] = ((_iota((DH, HD), 1) // H) == _iota((DH, HD), 0)).astype(_BF16)
        x_cp.wait()
        gate_cp.wait()

    NJ = DM // DH

    def p_bq(half):
        def run():
            if half == 0:
                wait_all(bwq_v, 0)
            js = range(half * (NJ // 2), (half + 1) * (NJ // 2))
            part = heads_to_rows(x_rows(), bwq_v, js)
            if half == 0:
                qb_ref[...] = part
            else:
                qb_ref[...] = qb_ref[...] + part
        return run

    def p_aq():
        wait_all(wq_v, 3)
        t = _dot(x_rows(), wq_v[...])
        qa = jnp.zeros((NR, DH), _F32)
        for u in range(H):
            qa = jnp.where(row_h == u, t[:, u * DH:(u + 1) * DH], qa)
        qa_ref[...] = qa.astype(_BF16).astype(_F32)

    def p_by(half):
        def run():
            if half == 0:
                wait_all(bwuk_v, 1)
            qb = qb_ref[...].astype(_BF16)
            nj = DC // DH
            for j in range(half * (nj // 2), (half + 1) * (nj // 2)):
                tt = _dot_nt(qb, bwuk_v[j * HD:(j + 1) * HD, :])
                tm = (tt * diag).astype(_BF16)
                y_ref[:, j * DH:(j + 1) * DH] = _dot_nt(tm, ebig[...])
        return run

    def p_scores(b, half):
        def run():
            if half == 0:
                wait_all(ckv_v.at[b], 6 + b)
            yb = y_ref[b * H:(b + 1) * H, :].astype(_BF16)
            ks = slice(half * (S // 2), (half + 1) * (S // 2))
            sb_ref[:, ks] = _dot_nt(yb, ckv_v[b, ks, :]) * scale
        return run

    def p_softmax(b):
        def run():
            s = sb_ref[...]
            m = jnp.max(s, axis=-1, keepdims=True)
            p = jnp.exp(s - m)
            sb_ref[...] = p / jnp.sum(p, axis=-1, keepdims=True)
        return run

    def p_ctx(b):
        def run():
            y_ref[b * H:(b + 1) * H, :] = _dot(sb_ref[...].astype(_BF16), ckv_v[b])
        return run

    def p_buv(half):
        def run():
            if half == 0:
                wait_all(bwuv_v, 2)
            nj = DC // DH
            js = range(half * (nj // 2), (half + 1) * (nj // 2))
            part = heads_to_rows(y_ref[...].astype(_BF16), bwuv_v, js)
            if half == 0:
                qb_ref[...] = part
            else:
                qb_ref[...] = qb_ref[...] + part
        return run

    def p_bo():
        wait_all(bwo_v, 5)
        ctx_d = qb_ref[...].astype(_BF16).astype(_F32)
        lz = jnp.concatenate(
            [jnp.where(row_h == u, ctx_d, 0.0) for u in range(H)], axis=1).astype(_BF16)
        zb = _dot(lz, bwo_v[...])
        row8 = _iota((8, DM), 0)
        out_b = jnp.zeros((8, DM), _F32)
        for b in range(NB):
            sb = jnp.sum(zb[b * H:(b + 1) * H, :], axis=0, keepdims=True)
            out_b = jnp.where(row8 == b, sb, out_b)
        bmix_ref[...] = out_b

    def p_gate():
        row8 = _iota((8, DM), 0)
        xv = x_ref[...].astype(_F32)
        x8 = jnp.zeros((8, DM), _F32)
        for b in range(NB):
            x8 = jnp.where(row8 == b, xv[b:b + 1, :], x8)
        gate = jax.nn.sigmoid(jnp.sum(
            x8 * gate_ref[...].astype(_F32).reshape(1, DM), axis=-1, keepdims=True))
        gmix_ref[...] = jnp.broadcast_to(gate, (8, DM))
        outa_ref[...] = jnp.zeros((8, DM), _F32)

    def p_wo():
        wait_all(wo_v, 4)

    NLT = KB // DH

    def fold(a):
        return [a[:, t * DH:(t + 1) * DH] for t in range(NLT)]

    def k_unit(g, b, slot):
        for hh in range(GH):
            q = jnp.broadcast_to(qa_ref[pl.ds(g * GH + hh, 1), :], (8, DH)).astype(_BF16)
            s = _dot_nt(q, ring[slot, hh]) * scale
            s_buf[hh, b] = s
            m = m_ref[hh]
            for t in fold(s):
                m = jnp.maximum(m, t)
            m_ref[hh] = m

    def v_probs(b):
        ps = []
        for hh in range(GH):
            p = jnp.exp(s_buf[hh, b] - jnp.tile(m_ref[hh], (1, NLT)))
            l = l_ref[hh]
            for t in fold(p):
                l = l + t
            l_ref[hh] = l
            ps.append(p.astype(_BF16))
        return ps

    def v_matmul(ps, slot):
        for hh in range(GH):
            acc_ref[hh] = acc_ref[hh] + _dot(ps[hh], ring[slot, hh])

    def v_unit(b, slot):
        ps = v_probs(b)
        wait_kv(slot)
        v_matmul(ps, slot)

    def k_begin():
        m_ref[...] = jnp.full(m_ref.shape, -jnp.inf, _F32)

    def v_begin():
        for hh in range(GH):
            m = jnp.max(m_ref[hh], axis=-1, keepdims=True)
            m_ref[hh] = jnp.broadcast_to(m, (8, DH))
        l_ref[...] = jnp.zeros(l_ref.shape, _F32)
        acc_ref[...] = jnp.zeros(acc_ref.shape, _F32)

    def finish_heads(g, heads, accs, ls):
        row8d = _iota((8, DH), 0)
        bidx = (g * GH) // H
        h0 = (g * GH) % H
        out = outa_ref[...]
        for hh, acc, l in zip(heads, accs, ls):
            o = jnp.where(row8d == bidx, acc / l, 0.0).astype(_BF16)
            out = out + _dot(o, wo_v[_ds((h0 + hh) * DH, DH), :])
        outa_ref[...] = out

    def row_sums():
        return [jnp.sum(l_ref[hh], axis=-1, keepdims=True) for hh in range(GH)]

    def v_last_unit_fused(g, slot):
        ps = v_probs(NBATCH - 1)
        ls = row_sums()
        wait_kv(slot)
        accs = [acc_ref[hh] + _dot(ps[hh], ring[slot, hh]) for hh in range(GH)]
        finish_heads(g, range(GH), accs, ls)

    x_cp.start()
    gate_cp.start()
    for run in b_batches("wq", "wo"):
        run()
    pro = [p_const, p_gate, p_aq]
    for u in range(L):
        issue_kv(k_hbm, 0, u, u % L)
        if u < len(pro):
            pro[u]()
    for piece in pro[L:]:
        piece()

    extras = {}

    def attach(u, *fns):
        extras.setdefault(u, []).extend(fns)

    u = 0
    done_at = {}
    order = {
        0: (("bwq", "bwo"), ("bwuk", "bwuv"), ("ckv0",), ("ckv1",)),
        1: (("bwq", "bwo", "bwuk", "bwuv"), ("ckv0", "ckv1")),
        2: (("bwq", "bwuk", "bwo", "bwuv"), ("ckv0",), ("ckv1",)),
        3: (("bwq", "bwuk"), ("ckv0", "ckv1"), ("bwuv", "bwo")),
    }[_BORDER]
    done_at["wo"] = 0
    for names in order:
        for run in b_batches(*names):
            attach(u, run)
            u += 1
        for name in names:
            done_at[name] = u
    n_load_units = u

    def chain(u, pieces):
        for piece in pieces:
            attach(u, piece)
            u += 1
        return u
    u = chain(done_at["bwq"] + 1, [p_bq(0), p_bq(1)])
    u = chain(max(u, done_at["bwuk"] + 1), [p_by(0), p_by(1)])
    u = chain(max(u, done_at["ckv0"] + 1),
              [p_scores(0, 0), p_scores(0, 1), p_softmax(0), p_ctx(0)])
    u = chain(max(u, done_at["ckv1"] + 1),
              [p_scores(1, 0), p_scores(1, 1), p_softmax(1), p_ctx(1)])
    u = chain(max(u, done_at["bwuv"] + 1), [p_buv(0), p_buv(1)])
    u = chain(max(u, done_at["bwo"] + 1), [p_bo])
    assert u <= NG * 2 * NBATCH and n_load_units <= 2 * NBATCH * NG
    assert done_at["wo"] + 1 < 2 * NBATCH
    attach(done_at["wo"] + 1, p_wo)

    def run_extras(phase, lo, hi, g, b):
        for uu in sorted(extras):
            eg, ephase, eb = uu // (2 * NBATCH), (uu // NBATCH) % 2, uu % NBATCH
            if ephase == phase and lo <= eb < hi:
                for fn in extras[uu]:
                    pl.when(jnp.logical_and(g == eg, b == eb))(fn)

    def group_body(g, final):
        base = g * (2 * NBATCH)

        def slot_of(u):
            return (base + u) % L

        def extras_for(phase, lo, hi, b):
            if not final:
                run_extras(phase, lo, hi, g, b)

        k_begin()

        def k_same(b, c):
            wait_kv(slot_of(b))
            k_unit(g, b, slot_of(b))
            issue_kv(k_hbm, g, b + L, slot_of(b))
            extras_for(0, 0, NBATCH - L, b)
            return c
        lax.fori_loop(0, NBATCH - L, k_same, 0)

        def k_next(b, c):
            wait_kv(slot_of(b))
            k_unit(g, b, slot_of(b))
            issue_kv(v_hbm, g, b + L - NBATCH, slot_of(b))
            extras_for(0, NBATCH - L, NBATCH, b)
            return c
        lax.fori_loop(NBATCH - L, NBATCH, k_next, 0)

        v_begin()

        def v_same(b, c):
            v_unit(b, slot_of(NBATCH + b))
            issue_kv(v_hbm, g, b + L, slot_of(NBATCH + b))
            extras_for(1, 0, NBATCH - L, b)
            return c
        lax.fori_loop(0, NBATCH - L, v_same, 0)

        if final:
            def v_drain(b, c):
                v_unit(b, slot_of(NBATCH + b))
                return c
            lax.fori_loop(NBATCH - L, NBATCH - 1, v_drain, 0)
            v_last_unit_fused(g, slot_of(2 * NBATCH - 1))
        else:
            def v_next(b, c):
                v_unit(b, slot_of(NBATCH + b))
                issue_kv(k_hbm, g + 1, b + L - NBATCH, slot_of(NBATCH + b))
                extras_for(1, NBATCH - L, NBATCH, b)
                return c
            lax.fori_loop(NBATCH - L, NBATCH, v_next, 0)
            finish_heads(g, range(GH), [acc_ref[hh] for hh in range(GH)], row_sums())

    assert max(extras) < (NG - 1) * 2 * NBATCH

    def regular_group(g, c):
        group_body(g, False)
        return c
    lax.fori_loop(0, NG - 1, regular_group, 0)
    group_body(NG - 1, True)

    gate = gmix_ref[...]
    res = gate * outa_ref[...] + (1.0 - gate) * bmix_ref[...]
    out_ref[...] = res[0:NB, :].astype(out_ref.dtype)
    out_cp.start()
    out_cp.wait()


@jax.jit
def pallas_gated_mix__mha_block_cached__compressed_kv_cla__decode_kernel(
    A_x: jax.Array,
    A_k_cache: jax.Array,
    A_v_cache: jax.Array,
    A_wq: jax.Array,
    A_wo: jax.Array,
    B_x: jax.Array,
    B_c_kv: jax.Array,
    B_w_q: jax.Array,
    B_w_uk: jax.Array,
    B_w_uv: jax.Array,
    B_w_o: jax.Array,
    gate_w: jax.Array,
):
    del B_x
    B, H, S, DH = A_k_cache.shape
    DM = A_x.shape[-1]
    DC = B_c_kv.shape[-1]
    NR = B * H
    KB = (_NDESC * _CHUNK_BYTES) // (_GH * DH * 2)

    k = A_k_cache.reshape(NR, S, DH)
    v = A_v_cache.reshape(NR, S, DH)
    bwq = B_w_q.reshape(DM * H, DH)
    bwuk = B_w_uk.reshape(DC * H, DH)
    bwuv = B_w_uv.reshape(DC * H, DH)
    bwo = B_w_o.reshape(H * DH, DM)

    hbm = pl.BlockSpec(memory_space=pl.ANY)
    dt = A_k_cache.dtype

    out = pl.pallas_call(
        _kernel,
        out_shape=jax.ShapeDtypeStruct((B, DM), A_x.dtype),
        in_specs=[hbm] * 11,
        out_specs=hbm,
        scratch_shapes=[
            pltpu.VMEM((B, DM), A_x.dtype),
            pltpu.VMEM(gate_w.shape, gate_w.dtype),
            pltpu.VMEM((B, DM), A_x.dtype),
            pltpu.VMEM((_NSLOT, _GH, KB, DH), dt),
            pltpu.VMEM(A_wq.shape, dt),
            pltpu.VMEM(A_wo.shape, dt),
            pltpu.VMEM(B_c_kv.shape, dt),
            pltpu.VMEM(bwq.shape, dt),
            pltpu.VMEM(bwuk.shape, dt),
            pltpu.VMEM(bwuv.shape, dt),
            pltpu.VMEM(bwo.shape, dt),
            pltpu.VMEM((DH, H * DH), _BF16),
            pltpu.VMEM((NR, DH), _F32),
            pltpu.VMEM((NR, DH), _F32),
            pltpu.VMEM((NR, DC), _F32),
            pltpu.VMEM((H, S), _F32),
            pltpu.VMEM((8, DM), _F32),
            pltpu.VMEM((8, DM), _F32),
            pltpu.VMEM((_GH, S // KB, 8, KB), _F32),
            pltpu.VMEM((_GH, 8, DH), _F32),
            pltpu.VMEM((_GH, 8, DH), _F32),
            pltpu.VMEM((_GH, 8, DH), _F32),
            pltpu.VMEM((8, DM), _F32),
            pltpu.SemaphoreType.DMA((_NSLOT,)),
            pltpu.SemaphoreType.DMA((9 + B,)),
        ],
        compiler_params=pltpu.CompilerParams(vmem_limit_bytes=100 * 1024 * 1024),
    )(A_x.reshape(B, DM), gate_w, k, v, A_wq, A_wo, B_c_kv, bwq, bwuk, bwuv, bwo)
    return out.reshape(B, 1, DM)
```

```python
import jax
import jax.numpy as jnp
from jax import lax
import jax.experimental.pallas as pl
import jax.experimental.pallas.tpu as pltpu

_NT = (((1,), (1,)), ((), ()))
_F32 = jnp.float32
_BF16 = jnp.bfloat16

_CHUNK_BYTES = 32 * 1024
_NDESC = 64
_GH = 16
_NSLOT = 3
_STREAM_BYTES = 1024 * 1024

_SEM = {"bwq": 0, "bwuk": 1, "bwuv": 2, "wq": 3, "wo": 4, "bwo": 5,
        "ckv0": 6, "ckv1": 7, "x": 8, "gate": 9, "out": 10}


def _dot(a, b):
    return jnp.dot(a, b, preferred_element_type=_F32)


def _dot_nt(a, b):
    return lax.dot_general(a, b, _NT, preferred_element_type=_F32)


def _iota(shape, dim):
    return lax.broadcasted_iota(jnp.int32, shape, dim)


def _ds(start, size):
    return pl.ds(pl.multiple_of(start, size), size)


def _kernel(
    x_hbm, gate_hbm, k_hbm, v_hbm, wq_hbm, wo_hbm, ckv_hbm,
    bwq_hbm, bwuk_hbm, bwuv_hbm, bwo_hbm,
    out_hbm,
    x_ref, gate_ref, out_ref, ring,
    wq_v, wo_v, ckv_v, bwq_v, bwuk_v, bwuv_v, bwo_v,
    ebig, qa_ref, qb_ref, y_ref, sb_ref, gmix_ref, bmix_ref,
    s_buf, m_ref, l_ref, acc_ref, outa_ref,
    ring_sems, w_sems,
):
    NR, S, DH = k_hbm.shape
    NB = ckv_hbm.shape[0]
    H = NR // NB
    DM = x_ref.shape[-1]
    DC = ckv_hbm.shape[-1]
    scale = DH ** -0.5

    GH = _GH
    NG = NR // GH
    KB = ring.shape[2]
    NBATCH = S // KB
    CR = _CHUNK_BYTES // (2 * DH)
    L = _NSLOT
    SCH = _STREAM_BYTES // _CHUNK_BYTES
    TW = 128
    TH = TW * H

    def b_streams(name):
        src, dst = {
            "bwq": (bwq_hbm, bwq_v), "bwuk": (bwuk_hbm, bwuk_v), "bwuv": (bwuv_hbm, bwuv_v),
            "wq": (wq_hbm, wq_v), "wo": (wo_hbm, wo_v), "bwo": (bwo_hbm, bwo_v),
            "ckv0": (ckv_hbm.at[0], ckv_v.at[0]), "ckv1": (ckv_hbm.at[1], ckv_v.at[1]),
        }[name]
        sem = w_sems.at[_SEM[name]]
        cols = min(src.shape[1], _CHUNK_BYTES // (2 * 16))
        rows = _CHUNK_BYTES // (2 * cols)
        ncb = src.shape[1] // cols
        srows = (SCH // ncb) * rows

        def mk(s):
            def cp(j):
                if ncb == 1:
                    idx = (_ds(s * srows + j * rows, rows),)
                else:
                    idx = (_ds(s * srows + (j // ncb) * rows, rows), _ds((j % ncb) * cols, cols))
                return pltpu.make_async_copy(src.at[idx], dst.at[idx], sem)
            return cp
        return [mk(s) for s in range(src.shape[0] // srows)]

    def b_batches(*names):
        streams = [cp for name in names for cp in b_streams(name)]
        jb = _NDESC // len(streams)

        def mk(j0):
            def run():
                def body(j, c):
                    for i, cp in enumerate(streams):
                        cp(j).start(priority=i % 2)
                    return c
                lax.fori_loop(j0, j0 + jb, body, 0)
            return run
        return [mk(j0) for j0 in range(0, SCH, jb)]

    def wait_all(ref, name):
        pltpu.make_async_copy(ref, ref, w_sems.at[_SEM[name]]).wait()

    def issue_kv(src, g, b, slot):
        for j in range(KB // CR):
            for hh in range(GH):
                pltpu.make_async_copy(
                    src.at[g * GH + hh, _ds(b * KB + j * CR, CR)],
                    ring.at[slot, hh, pl.ds(j * CR, CR)],
                    ring_sems.at[slot],
                ).start(priority=hh % 2)

    def wait_kv(slot):
        pltpu.make_async_copy(ring.at[slot], ring.at[slot], ring_sems.at[slot]).wait()

    x_cp = pltpu.make_async_copy(x_hbm, x_ref, w_sems.at[_SEM["x"]])
    gate_cp = pltpu.make_async_copy(gate_hbm, gate_ref, w_sems.at[_SEM["gate"]])
    out_cp = pltpu.make_async_copy(out_ref, out_hbm, w_sems.at[_SEM["out"]])

    diag128 = ((_iota((NR, TW), 1) % H) == (_iota((NR, TW), 0) % H)).astype(_F32)
    diag = jnp.tile(diag128, (1, TH // TW))
    row_h = _iota((NR, DH), 0) % H

    def x_rows():
        xv = x_ref[...]
        return jnp.concatenate(
            [jnp.broadcast_to(xv[b:b + 1, :], (H, DM)) for b in range(NB)], axis=0)

    def heads_to_rows(a, w_ref, js):
        acc = None
        for j in js:
            aexp = _dot(a[:, j * TW:(j + 1) * TW], ebig[...])
            lhs = (aexp * diag).astype(_BF16)
            part = _dot(lhs, w_ref[j * TH:(j + 1) * TH, :])
            acc = part if acc is None else acc + part
        return acc

    def tiles(n, half):
        return range(half * (n // 2), (half + 1) * (n // 2))

    def p_const():
        ebig[...] = ((_iota((TW, TH), 1) // H) == _iota((TW, TH), 0)).astype(_BF16)
        x_cp.wait()
        gate_cp.wait()

    def p_gate():
        row8 = _iota((8, DM), 0)
        xv = x_ref[...].astype(_F32)
        x8 = jnp.zeros((8, DM), _F32)
        for b in range(NB):
            x8 = jnp.where(row8 == b, xv[b:b + 1, :], x8)
        gate = jax.nn.sigmoid(jnp.sum(
            x8 * gate_ref[...].astype(_F32).reshape(1, DM), axis=-1, keepdims=True))
        gmix_ref[...] = jnp.broadcast_to(gate, (8, DM))
        outa_ref[...] = jnp.zeros((8, DM), _F32)

    def p_aq():
        wait_all(wq_v, "wq")
        t = _dot(x_rows(), wq_v[...])
        qa = jnp.zeros((NR, DH), _F32)
        for u in range(H):
            qa = jnp.where(row_h == u, t[:, u * DH:(u + 1) * DH], qa)
        qa_ref[...] = qa.astype(_BF16).astype(_F32)

    def p_bq(half):
        def run():
            if half == 0:
                wait_all(bwq_v, "bwq")
            part = heads_to_rows(x_rows(), bwq_v, tiles(DM // TW, half))
            qb_ref[...] = part if half == 0 else qb_ref[...] + part
        return run

    def p_by(half):
        def run():
            if half == 0:
                wait_all(bwuk_v, "bwuk")
            qb = qb_ref[...].astype(_BF16)
            for j in tiles(DC // TW, half):
                tt = _dot_nt(qb, bwuk_v[j * TH:(j + 1) * TH, :])
                tm = (tt * diag).astype(_BF16)
                y_ref[:, j * TW:(j + 1) * TW] = _dot_nt(tm, ebig[...])
        return run

    def p_scores(b, half):
        def run():
            if half == 0:
                wait_all(ckv_v.at[b], "ckv%d" % b)
            yb = y_ref[b * H:(b + 1) * H, :].astype(_BF16)
            ks = slice(half * (S // 2), (half + 1) * (S // 2))
            sb_ref[:, ks] = _dot_nt(yb, ckv_v[b, ks, :]) * scale
        return run

    def p_softmax(b):
        def run():
            s = sb_ref[...]
            m = jnp.max(s, axis=-1, keepdims=True)
            p = jnp.exp(s - m)
            sb_ref[...] = p / jnp.sum(p, axis=-1, keepdims=True)
        return run

    def p_ctx(b):
        def run():
            y_ref[b * H:(b + 1) * H, :] = _dot(sb_ref[...].astype(_BF16), ckv_v[b])
        return run

    def p_buv(half):
        def run():
            if half == 0:
                wait_all(bwuv_v, "bwuv")
            part = heads_to_rows(y_ref[...].astype(_BF16), bwuv_v, tiles(DC // TW, half))
            qb_ref[...] = part if half == 0 else qb_ref[...] + part
        return run

    def p_bo():
        wait_all(bwo_v, "bwo")
        ctx_d = qb_ref[...].astype(_BF16).astype(_F32)
        lz = jnp.concatenate(
            [jnp.where(row_h == u, ctx_d, 0.0) for u in range(H)], axis=1).astype(_BF16)
        zb = _dot(lz, bwo_v[...])
        row8 = _iota((8, DM), 0)
        out_b = jnp.zeros((8, DM), _F32)
        for b in range(NB):
            sb = jnp.sum(zb[b * H:(b + 1) * H, :], axis=0, keepdims=True)
            out_b = jnp.where(row8 == b, sb, out_b)
        bmix_ref[...] = out_b

    def p_wo():
        wait_all(wo_v, "wo")

    NLT = KB // DH

    def lane_tiles(a):
        return [a[:, t * DH:(t + 1) * DH] for t in range(NLT)]

    def k_begin():
        m_ref[...] = jnp.full(m_ref.shape, -jnp.inf, _F32)

    def k_unit(g, b, slot):
        for hh in range(GH):
            q = jnp.broadcast_to(qa_ref[pl.ds(g * GH + hh, 1), :], (8, DH)).astype(_BF16)
            s = _dot_nt(q, ring[slot, hh]) * scale
            s_buf[hh, b] = s
            m = m_ref[hh]
            for t in lane_tiles(s):
                m = jnp.maximum(m, t)
            m_ref[hh] = m

    def v_begin():
        for hh in range(GH):
            m = jnp.max(m_ref[hh], axis=-1, keepdims=True)
            m_ref[hh] = jnp.broadcast_to(m, (8, DH))
        l_ref[...] = jnp.zeros(l_ref.shape, _F32)
        acc_ref[...] = jnp.zeros(acc_ref.shape, _F32)

    def v_probs(b):
        ps = []
        for hh in range(GH):
            p = jnp.exp(s_buf[hh, b] - jnp.tile(m_ref[hh], (1, NLT)))
            l = l_ref[hh]
            for t in lane_tiles(p):
                l = l + t
            l_ref[hh] = l
            ps.append(p.astype(_BF16))
        return ps

    def v_unit(b, slot):
        ps = v_probs(b)
        wait_kv(slot)
        for hh in range(GH):
            acc_ref[hh] = acc_ref[hh] + _dot(ps[hh], ring[slot, hh])

    def row_sums():
        return [jnp.sum(l_ref[hh], axis=-1, keepdims=True) for hh in range(GH)]

    def finish_heads(g, accs, ls):
        row8d = _iota((8, DH), 0)
        bidx = (g * GH) // H
        h0 = (g * GH) % H
        out = outa_ref[...]
        for hh in range(GH):
            o = jnp.where(row8d == bidx, accs[hh] / ls[hh], 0.0).astype(_BF16)
            out = out + _dot(o, wo_v[_ds((h0 + hh) * DH, DH), :])
        outa_ref[...] = out

    def v_last_unit_fused(g, slot):
        ps = v_probs(NBATCH - 1)
        ls = row_sums()
        wait_kv(slot)
        accs = [acc_ref[hh] + _dot(ps[hh], ring[slot, hh]) for hh in range(GH)]
        finish_heads(g, accs, ls)

    for i, run in enumerate(b_batches("wq", "wo")):
        run()
        if i == 0:
            x_cp.start(priority=0)
            gate_cp.start(priority=1)
    pro = [p_const, p_gate, p_aq]
    for u in range(L):
        issue_kv(k_hbm, 0, u, u % L)
        if u < len(pro):
            pro[u]()
    for piece in pro[L:]:
        piece()

    extras = {}

    def attach(u, fn):
        extras.setdefault(u, []).append(fn)

    u = 0
    loaded = {}
    for names in (("bwq", "bwo", "bwuk", "bwuv"), ("ckv0", "ckv1")):
        for run in b_batches(*names):
            attach(u, run)
            u += 1
        for name in names:
            loaded[name] = u

    def chain(u, pieces):
        for piece in pieces:
            attach(u, piece)
            u += 1
        return u

    attach(1, p_wo)
    u = chain(loaded["bwq"] + 1, [p_bq(0), p_bq(1)])
    u = chain(max(u, loaded["bwuk"] + 1), [p_by(0), p_by(1)])
    for b in range(NB):
        u = chain(max(u, loaded["ckv%d" % b] + 1),
                  [p_scores(b, 0), p_scores(b, 1), p_softmax(b), p_ctx(b)])
    u = chain(max(u, loaded["bwuv"] + 1), [p_buv(0), p_buv(1)])
    u = chain(max(u, loaded["bwo"] + 1), [p_bo])
    assert max(extras) < (NG - 1) * 2 * NBATCH

    def run_extras(phase, lo, hi, g, b):
        for uu in sorted(extras):
            eg, ephase, eb = uu // (2 * NBATCH), (uu // NBATCH) % 2, uu % NBATCH
            if ephase == phase and lo <= eb < hi:
                for fn in extras[uu]:
                    pl.when(jnp.logical_and(g == eg, b == eb))(fn)

    def group_body(g, final):
        base = g * (2 * NBATCH)

        def slot_of(u):
            return (base + u) % L

        def refill(src, gg, bb, slot, phase, lo, hi, b):
            issue_kv(src, gg, bb, slot)
            if not final:
                run_extras(phase, lo, hi, g, b)

        k_begin()

        def k_same(b, c):
            wait_kv(slot_of(b))
            k_unit(g, b, slot_of(b))
            refill(k_hbm, g, b + L, slot_of(b), 0, 0, NBATCH - L, b)
            return c
        lax.fori_loop(0, NBATCH - L, k_same, 0)

        def k_next(b, c):
            wait_kv(slot_of(b))
            k_unit(g, b, slot_of(b))
            refill(v_hbm, g, b + L - NBATCH, slot_of(b), 0, NBATCH - L, NBATCH, b)
            return c
        lax.fori_loop(NBATCH - L, NBATCH, k_next, 0)

        v_begin()

        def v_same(b, c):
            v_unit(b, slot_of(NBATCH + b))
            refill(v_hbm, g, b + L, slot_of(NBATCH + b), 1, 0, NBATCH - L, b)
            return c
        lax.fori_loop(0, NBATCH - L, v_same, 0)

        if final:
            def v_drain(b, c):
                v_unit(b, slot_of(NBATCH + b))
                return c
            lax.fori_loop(NBATCH - L, NBATCH - 1, v_drain, 0)
            v_last_unit_fused(g, slot_of(2 * NBATCH - 1))
        else:
            def v_next(b, c):
                v_unit(b, slot_of(NBATCH + b))
                refill(k_hbm, g + 1, b + L - NBATCH, slot_of(NBATCH + b),
                       1, NBATCH - L, NBATCH, b)
                return c
            lax.fori_loop(NBATCH - L, NBATCH, v_next, 0)
            finish_heads(g, [acc_ref[hh] for hh in range(GH)], row_sums())

    def regular_group(g, c):
        group_body(g, False)
        return c
    lax.fori_loop(0, NG - 1, regular_group, 0)
    group_body(NG - 1, True)

    gate = gmix_ref[...]
    res = gate * outa_ref[...] + (1.0 - gate) * bmix_ref[...]
    out_ref[...] = res[0:NB, :].astype(out_ref.dtype)
    out_cp.start()
    out_cp.wait()


@jax.jit
def pallas_gated_mix__mha_block_cached__compressed_kv_cla__decode_kernel(
    A_x: jax.Array,
    A_k_cache: jax.Array,
    A_v_cache: jax.Array,
    A_wq: jax.Array,
    A_wo: jax.Array,
    B_x: jax.Array,
    B_c_kv: jax.Array,
    B_w_q: jax.Array,
    B_w_uk: jax.Array,
    B_w_uv: jax.Array,
    B_w_o: jax.Array,
    gate_w: jax.Array,
):
    del B_x
    B, H, S, DH = A_k_cache.shape
    DM = A_x.shape[-1]
    DC = B_c_kv.shape[-1]
    NR = B * H
    KB = (_NDESC * _CHUNK_BYTES) // (_GH * DH * 2)
    assert B == 2 and A_x.shape[1] == 1

    k = A_k_cache.reshape(NR, S, DH)
    v = A_v_cache.reshape(NR, S, DH)
    bwq = B_w_q.reshape(DM * H, DH)
    bwuk = B_w_uk.reshape(DC * H, DH)
    bwuv = B_w_uv.reshape(DC * H, DH)
    bwo = B_w_o.reshape(H * DH, DM)

    hbm = pl.BlockSpec(memory_space=pl.ANY)
    dt = A_k_cache.dtype

    out = pl.pallas_call(
        _kernel,
        out_shape=jax.ShapeDtypeStruct((B, DM), A_x.dtype),
        in_specs=[hbm] * 11,
        out_specs=hbm,
        scratch_shapes=[
            pltpu.VMEM((B, DM), A_x.dtype),
            pltpu.VMEM(gate_w.shape, gate_w.dtype),
            pltpu.VMEM((B, DM), A_x.dtype),
            pltpu.VMEM((_NSLOT, _GH, KB, DH), dt),
            pltpu.VMEM(A_wq.shape, dt),
            pltpu.VMEM(A_wo.shape, dt),
            pltpu.VMEM(B_c_kv.shape, dt),
            pltpu.VMEM(bwq.shape, dt),
            pltpu.VMEM(bwuk.shape, dt),
            pltpu.VMEM(bwuv.shape, dt),
            pltpu.VMEM(bwo.shape, dt),
            pltpu.VMEM((128, 128 * H), _BF16),
            pltpu.VMEM((NR, DH), _F32),
            pltpu.VMEM((NR, DH), _F32),
            pltpu.VMEM((NR, DC), _F32),
            pltpu.VMEM((H, S), _F32),
            pltpu.VMEM((8, DM), _F32),
            pltpu.VMEM((8, DM), _F32),
            pltpu.VMEM((_GH, S // KB, 8, KB), _F32),
            pltpu.VMEM((_GH, 8, DH), _F32),
            pltpu.VMEM((_GH, 8, DH), _F32),
            pltpu.VMEM((_GH, 8, DH), _F32),
            pltpu.VMEM((8, DM), _F32),
            pltpu.SemaphoreType.DMA((_NSLOT,)),
            pltpu.SemaphoreType.DMA((len(_SEM),)),
        ],
        compiler_params=pltpu.CompilerParams(vmem_limit_bytes=100 * 1024 * 1024),
    )(A_x.reshape(B, DM), gate_w, k, v, A_wq, A_wo, B_c_kv, bwq, bwuk, bwuv, bwo)
    return out.reshape(B, 1, DM)
```

```python
import jax
import jax.numpy as jnp
from jax import lax
import jax.experimental.pallas as pl
import jax.experimental.pallas.tpu as pltpu

_NT = (((1,), (1,)), ((), ()))
_F32 = jnp.float32
_BF16 = jnp.bfloat16

_CHUNK_BYTES = 32 * 1024
_NDESC = 64
_GH = 16
_NSLOT = 3
_STREAM_BYTES = 1024 * 1024

_SEM = {"bwq": 0, "bwuk": 1, "bwuv": 2, "wq": 3, "wo": 4, "bwo": 5,
        "ckv0": 6, "ckv1": 7, "x": 8, "gate": 9, "out": 10}


def _dot(a, b):
    return jnp.dot(a, b, preferred_element_type=_F32)


def _dot_nt(a, b):
    return lax.dot_general(a, b, _NT, preferred_element_type=_F32)


def _iota(shape, dim):
    return lax.broadcasted_iota(jnp.int32, shape, dim)


def _ds(start, size):
    return pl.ds(pl.multiple_of(start, size), size)


def _kernel(
    x_hbm, gate_hbm, k_hbm, v_hbm, wq_hbm, wo_hbm, ckv_hbm,
    bwq_hbm, bwuk_hbm, bwuv_hbm, bwo_hbm,
    out_hbm,
    x_ref, gate_ref, out_ref, ring,
    wq_v, wo_v, ckv_v, bwq_v, bwuk_v, bwuv_v, bwo_v,
    ebig, qa_ref, qb_ref, y_ref, sb_ref, gmix_ref, bmix_ref,
    s_buf, m_ref, l_ref, acc_ref, outa_ref,
    ring_sems, w_sems,
):
    NR, S, DH = k_hbm.shape
    NB = ckv_hbm.shape[0]
    H = NR // NB
    DM = x_ref.shape[-1]
    DC = ckv_hbm.shape[-1]
    scale = DH ** -0.5

    GH = _GH
    NG = NR // GH
    KB = ring.shape[2]
    NBATCH = S // KB
    CR = _CHUNK_BYTES // (2 * DH)
    L = _NSLOT
    SCH = _STREAM_BYTES // _CHUNK_BYTES
    TW = 128
    TH = TW * H

    def row_of(g, hh):
        return hh * NG + g

    def b_streams(name):
        src, dst = {
            "bwq": (bwq_hbm, bwq_v), "bwuk": (bwuk_hbm, bwuk_v), "bwuv": (bwuv_hbm, bwuv_v),
            "wq": (wq_hbm, wq_v), "wo": (wo_hbm, wo_v), "bwo": (bwo_hbm, bwo_v),
            "ckv0": (ckv_hbm.at[0], ckv_v.at[0]), "ckv1": (ckv_hbm.at[1], ckv_v.at[1]),
        }[name]
        sem = w_sems.at[_SEM[name]]
        cols = min(src.shape[1], _CHUNK_BYTES // (2 * 16))
        rows = _CHUNK_BYTES // (2 * cols)
        ncb = src.shape[1] // cols
        srows = (SCH // ncb) * rows

        def mk(s):
            def cp(j):
                if ncb == 1:
                    idx = (_ds(s * srows + j * rows, rows),)
                else:
                    idx = (_ds(s * srows + (j // ncb) * rows, rows), _ds((j % ncb) * cols, cols))
                return pltpu.make_async_copy(src.at[idx], dst.at[idx], sem)
            return cp
        return [mk(s) for s in range(src.shape[0] // srows)]

    def b_batches(*names):
        streams = [cp for name in names for cp in b_streams(name)]
        jb = _NDESC // len(streams)

        def mk(j0):
            def run():
                def body(j, c):
                    for i, cp in enumerate(streams):
                        cp(j).start(priority=i % 2)
                    return c
                lax.fori_loop(j0, j0 + jb, body, 0)
            return run
        return [mk(j0) for j0 in range(0, SCH, jb)]

    def wait_all(ref, name):
        pltpu.make_async_copy(ref, ref, w_sems.at[_SEM[name]]).wait()

    def issue_kv(src, g, b, slot):
        for j in range(KB // CR):
            for hh in range(GH):
                pltpu.make_async_copy(
                    src.at[row_of(g, hh), _ds(b * KB + j * CR, CR)],
                    ring.at[slot, hh, pl.ds(j * CR, CR)],
                    ring_sems.at[slot],
                ).start(priority=hh % 2)

    def wait_kv(slot):
        pltpu.make_async_copy(ring.at[slot], ring.at[slot], ring_sems.at[slot]).wait()

    x_cp = pltpu.make_async_copy(x_hbm, x_ref, w_sems.at[_SEM["x"]])
    gate_cp = pltpu.make_async_copy(gate_hbm, gate_ref, w_sems.at[_SEM["gate"]])
    out_cp = pltpu.make_async_copy(out_ref, out_hbm, w_sems.at[_SEM["out"]])

    diag128 = ((_iota((NR, TW), 1) % H) == (_iota((NR, TW), 0) % H)).astype(_F32)
    diag = jnp.tile(diag128, (1, TH // TW))
    row_h = _iota((NR, DH), 0) % H

    def x_rows():
        xv = x_ref[...]
        return jnp.concatenate(
            [jnp.broadcast_to(xv[b:b + 1, :], (H, DM)) for b in range(NB)], axis=0)

    def heads_to_rows(a, w_ref, js):
        acc = None
        for j in js:
            aexp = _dot(a[:, j * TW:(j + 1) * TW], ebig[...])
            lhs = (aexp * diag).astype(_BF16)
            part = _dot(lhs, w_ref[j * TH:(j + 1) * TH, :])
            acc = part if acc is None else acc + part
        return acc

    def tiles(n, half):
        return range(half * (n // 2), (half + 1) * (n // 2))

    def p_const():
        ebig[...] = ((_iota((TW, TH), 1) // H) == _iota((TW, TH), 0)).astype(_BF16)
        x_cp.wait()
        gate_cp.wait()

    def p_gate():
        row8 = _iota((8, DM), 0)
        xv = x_ref[...].astype(_F32)
        x8 = jnp.zeros((8, DM), _F32)
        for b in range(NB):
            x8 = jnp.where(row8 == b, xv[b:b + 1, :], x8)
        gate = jax.nn.sigmoid(jnp.sum(
            x8 * gate_ref[...].astype(_F32).reshape(1, DM), axis=-1, keepdims=True))
        gmix_ref[...] = jnp.broadcast_to(gate, (8, DM))
        outa_ref[...] = jnp.zeros((8, DM), _F32)

    def p_aq():
        wait_all(wq_v, "wq")
        t = _dot(x_rows(), wq_v[...])
        qa = jnp.zeros((NR, DH), _F32)
        for u in range(H):
            qa = jnp.where(row_h == u, t[:, u * DH:(u + 1) * DH], qa)
        qa_ref[...] = qa.astype(_BF16).astype(_F32)

    def p_bq(half):
        def run():
            if half == 0:
                wait_all(bwq_v, "bwq")
            part = heads_to_rows(x_rows(), bwq_v, tiles(DM // TW, half))
            qb_ref[...] = part if half == 0 else qb_ref[...] + part
        return run

    def p_by(half):
        def run():
            if half == 0:
                wait_all(bwuk_v, "bwuk")
            qb = qb_ref[...].astype(_BF16)
            for j in tiles(DC // TW, half):
                tt = _dot_nt(qb, bwuk_v[j * TH:(j + 1) * TH, :])
                tm = (tt * diag).astype(_BF16)
                y_ref[:, j * TW:(j + 1) * TW] = _dot_nt(tm, ebig[...])
        return run

    def p_scores(b, half):
        def run():
            if half == 0:
                wait_all(ckv_v.at[b], "ckv%d" % b)
            yb = y_ref[b * H:(b + 1) * H, :].astype(_BF16)
            ks = slice(half * (S // 2), (half + 1) * (S // 2))
            sb_ref[:, ks] = _dot_nt(yb, ckv_v[b, ks, :]) * scale
        return run

    def p_softmax(b):
        def run():
            s = sb_ref[...]
            m = jnp.max(s, axis=-1, keepdims=True)
            p = jnp.exp(s - m)
            sb_ref[...] = p / jnp.sum(p, axis=-1, keepdims=True)
        return run

    def p_ctx(b):
        def run():
            y_ref[b * H:(b + 1) * H, :] = _dot(sb_ref[...].astype(_BF16), ckv_v[b])
        return run

    def p_buv(half):
        def run():
            if half == 0:
                wait_all(bwuv_v, "bwuv")
            part = heads_to_rows(y_ref[...].astype(_BF16), bwuv_v, tiles(DC // TW, half))
            qb_ref[...] = part if half == 0 else qb_ref[...] + part
        return run

    def p_bo():
        wait_all(bwo_v, "bwo")
        ctx_d = qb_ref[...].astype(_BF16).astype(_F32)
        lz = jnp.concatenate(
            [jnp.where(row_h == u, ctx_d, 0.0) for u in range(H)], axis=1).astype(_BF16)
        zb = _dot(lz, bwo_v[...])
        row8 = _iota((8, DM), 0)
        out_b = jnp.zeros((8, DM), _F32)
        for b in range(NB):
            sb = jnp.sum(zb[b * H:(b + 1) * H, :], axis=0, keepdims=True)
            out_b = jnp.where(row8 == b, sb, out_b)
        bmix_ref[...] = out_b

    def p_wo():
        wait_all(wo_v, "wo")

    NLT = KB // DH

    def lane_tiles(a):
        return [a[:, t * DH:(t + 1) * DH] for t in range(NLT)]

    def k_begin():
        m_ref[...] = jnp.full(m_ref.shape, -jnp.inf, _F32)

    def k_unit(g, b, slot):
        for hh in range(GH):
            q = jnp.broadcast_to(qa_ref[pl.ds(row_of(g, hh), 1), :], (8, DH)).astype(_BF16)
            s = _dot_nt(q, ring[slot, hh]) * scale
            s_buf[hh, b] = s
            m = m_ref[hh]
            for t in lane_tiles(s):
                m = jnp.maximum(m, t)
            m_ref[hh] = m

    def v_begin():
        for hh in range(GH):
            m = jnp.max(m_ref[hh], axis=-1, keepdims=True)
            m_ref[hh] = jnp.broadcast_to(m, (8, DH))
        l_ref[...] = jnp.zeros(l_ref.shape, _F32)
        acc_ref[...] = jnp.zeros(acc_ref.shape, _F32)

    def v_probs(b):
        ps = []
        for hh in range(GH):
            p = jnp.exp(s_buf[hh, b] - jnp.tile(m_ref[hh], (1, NLT)))
            l = l_ref[hh]
            for t in lane_tiles(p):
                l = l + t
            l_ref[hh] = l
            ps.append(p.astype(_BF16))
        return ps

    def v_unit(b, slot):
        ps = v_probs(b)
        wait_kv(slot)
        for hh in range(GH):
            acc_ref[hh] = acc_ref[hh] + _dot(ps[hh], ring[slot, hh])

    def row_sums():
        return [jnp.sum(l_ref[hh], axis=-1, keepdims=True) for hh in range(GH)]

    def finish_heads(g, accs, ls):
        row8d = _iota((8, DH), 0)
        out = outa_ref[...]
        for hh in range(GH):
            r = row_of(g, hh)
            o = jnp.where(row8d == r // H, accs[hh] / ls[hh], 0.0).astype(_BF16)
            out = out + _dot(o, wo_v[_ds((r % H) * DH, DH), :])
        outa_ref[...] = out

    def v_last_unit_fused(g, slot):
        ps = v_probs(NBATCH - 1)
        ls = row_sums()
        wait_kv(slot)
        accs = [acc_ref[hh] + _dot(ps[hh], ring[slot, hh]) for hh in range(GH)]
        finish_heads(g, accs, ls)

    for i, run in enumerate(b_batches("wq", "wo")):
        run()
        if i == 0:
            x_cp.start(priority=0)
            gate_cp.start(priority=1)
    pro = [p_const, p_gate, p_aq]
    for u in range(L):
        issue_kv(k_hbm, 0, u, u % L)
        if u < len(pro):
            pro[u]()
    for piece in pro[L:]:
        piece()

    extras = {}

    def attach(u, fn):
        extras.setdefault(u, []).append(fn)

    u = 0
    loaded = {}
    for names in (("bwq", "bwo", "bwuk", "bwuv"), ("ckv0", "ckv1")):
        for run in b_batches(*names):
            attach(u, run)
            u += 1
        for name in names:
            loaded[name] = u

    def chain(u, pieces):
        for piece in pieces:
            attach(u, piece)
            u += 1
        return u

    attach(1, p_wo)
    u = chain(loaded["bwq"] + 1, [p_bq(0), p_bq(1)])
    u = chain(max(u, loaded["bwuk"] + 1), [p_by(0), p_by(1)])
    for b in range(NB):
        u = chain(max(u, loaded["ckv%d" % b] + 1),
                  [p_scores(b, 0), p_scores(b, 1), p_softmax(b), p_ctx(b)])
    u = chain(max(u, loaded["bwuv"] + 1), [p_buv(0), p_buv(1)])
    u = chain(max(u, loaded["bwo"] + 1), [p_bo])
    assert max(extras) < (NG - 1) * 2 * NBATCH

    def run_extras(phase, lo, hi, g, b):
        for uu in sorted(extras):
            eg, ephase, eb = uu // (2 * NBATCH), (uu // NBATCH) % 2, uu % NBATCH
            if ephase == phase and lo <= eb < hi:
                for fn in extras[uu]:
                    pl.when(jnp.logical_and(g == eg, b == eb))(fn)

    def group_body(g, final):
        base = g * (2 * NBATCH)

        def slot_of(u):
            return (base + u) % L

        def refill(src, gg, bb, slot, phase, lo, hi, b):
            issue_kv(src, gg, bb, slot)
            if not final:
                run_extras(phase, lo, hi, g, b)

        k_begin()

        def k_same(b, c):
            wait_kv(slot_of(b))
            k_unit(g, b, slot_of(b))
            refill(k_hbm, g, b + L, slot_of(b), 0, 0, NBATCH - L, b)
            return c
        lax.fori_loop(0, NBATCH - L, k_same, 0)

        def k_next(b, c):
            wait_kv(slot_of(b))
            k_unit(g, b, slot_of(b))
            refill(v_hbm, g, b + L - NBATCH, slot_of(b), 0, NBATCH - L, NBATCH, b)
            return c
        lax.fori_loop(NBATCH - L, NBATCH, k_next, 0)

        v_begin()

        def v_same(b, c):
            v_unit(b, slot_of(NBATCH + b))
            refill(v_hbm, g, b + L, slot_of(NBATCH + b), 1, 0, NBATCH - L, b)
            return c
        lax.fori_loop(0, NBATCH - L, v_same, 0)

        if final:
            def v_drain(b, c):
                v_unit(b, slot_of(NBATCH + b))
                return c
            lax.fori_loop(NBATCH - L, NBATCH - 1, v_drain, 0)
            v_last_unit_fused(g, slot_of(2 * NBATCH - 1))
        else:
            def v_next(b, c):
                v_unit(b, slot_of(NBATCH + b))
                refill(k_hbm, g + 1, b + L - NBATCH, slot_of(NBATCH + b),
                       1, NBATCH - L, NBATCH, b)
                return c
            lax.fori_loop(NBATCH - L, NBATCH, v_next, 0)
            finish_heads(g, [acc_ref[hh] for hh in range(GH)], row_sums())

    def regular_group(g, c):
        group_body(g, False)
        return c
    lax.fori_loop(0, NG - 1, regular_group, 0)
    group_body(NG - 1, True)

    gate = gmix_ref[...]
    res = gate * outa_ref[...] + (1.0 - gate) * bmix_ref[...]
    out_ref[...] = res[0:NB, :].astype(out_ref.dtype)
    out_cp.start()
    out_cp.wait()


@jax.jit
def pallas_gated_mix__mha_block_cached__compressed_kv_cla__decode_kernel(
    A_x: jax.Array,
    A_k_cache: jax.Array,
    A_v_cache: jax.Array,
    A_wq: jax.Array,
    A_wo: jax.Array,
    B_x: jax.Array,
    B_c_kv: jax.Array,
    B_w_q: jax.Array,
    B_w_uk: jax.Array,
    B_w_uv: jax.Array,
    B_w_o: jax.Array,
    gate_w: jax.Array,
):
    del B_x
    B, H, S, DH = A_k_cache.shape
    DM = A_x.shape[-1]
    DC = B_c_kv.shape[-1]
    NR = B * H
    KB = (_NDESC * _CHUNK_BYTES) // (_GH * DH * 2)
    assert B == 2 and A_x.shape[1] == 1

    k = A_k_cache.reshape(NR, S, DH)
    v = A_v_cache.reshape(NR, S, DH)
    bwq = B_w_q.reshape(DM * H, DH)
    bwuk = B_w_uk.reshape(DC * H, DH)
    bwuv = B_w_uv.reshape(DC * H, DH)
    bwo = B_w_o.reshape(H * DH, DM)

    hbm = pl.BlockSpec(memory_space=pl.ANY)
    dt = A_k_cache.dtype

    out = pl.pallas_call(
        _kernel,
        out_shape=jax.ShapeDtypeStruct((B, DM), A_x.dtype),
        in_specs=[hbm] * 11,
        out_specs=hbm,
        scratch_shapes=[
            pltpu.VMEM((B, DM), A_x.dtype),
            pltpu.VMEM(gate_w.shape, gate_w.dtype),
            pltpu.VMEM((B, DM), A_x.dtype),
            pltpu.VMEM((_NSLOT, _GH, KB, DH), dt),
            pltpu.VMEM(A_wq.shape, dt),
            pltpu.VMEM(A_wo.shape, dt),
            pltpu.VMEM(B_c_kv.shape, dt),
            pltpu.VMEM(bwq.shape, dt),
            pltpu.VMEM(bwuk.shape, dt),
            pltpu.VMEM(bwuv.shape, dt),
            pltpu.VMEM(bwo.shape, dt),
            pltpu.VMEM((128, 128 * H), _BF16),
            pltpu.VMEM((NR, DH), _F32),
            pltpu.VMEM((NR, DH), _F32),
            pltpu.VMEM((NR, DC), _F32),
            pltpu.VMEM((H, S), _F32),
            pltpu.VMEM((8, DM), _F32),
            pltpu.VMEM((8, DM), _F32),
            pltpu.VMEM((_GH, S // KB, 8, KB), _F32),
            pltpu.VMEM((_GH, 8, DH), _F32),
            pltpu.VMEM((_GH, 8, DH), _F32),
            pltpu.VMEM((_GH, 8, DH), _F32),
            pltpu.VMEM((8, DM), _F32),
            pltpu.SemaphoreType.DMA((_NSLOT,)),
            pltpu.SemaphoreType.DMA((len(_SEM),)),
        ],
        compiler_params=pltpu.CompilerParams(vmem_limit_bytes=100 * 1024 * 1024),
    )(A_x.reshape(B, DM), gate_w, k, v, A_wq, A_wo, B_c_kv, bwq, bwuk, bwuv, bwo)
    return out.reshape(B, 1, DM)
```

```python
import jax
import jax.numpy as jnp
from jax import lax
import jax.experimental.pallas as pl
import jax.experimental.pallas.tpu as pltpu

_NT = (((1,), (1,)), ((), ()))
_F32 = jnp.float32
_BF16 = jnp.bfloat16

_CHUNK_BYTES = 32 * 1024
_NDESC = 64
_GH = 16
_NSLOT = 3
_STREAM_BYTES = 512 * 1024

_SEM = {"bwq": 0, "bwuk": 1, "bwuv": 2, "wq": 3, "wo": 4, "bwo": 5,
        "ckv0": 6, "ckv1": 7, "x": 8, "gate": 9, "out": 10}


def _dot(a, b):
    return jnp.dot(a, b, preferred_element_type=_F32)


def _dot_nt(a, b):
    return lax.dot_general(a, b, _NT, preferred_element_type=_F32)


def _iota(shape, dim):
    return lax.broadcasted_iota(jnp.int32, shape, dim)


def _ds(start, size):
    return pl.ds(pl.multiple_of(start, size), size)


def _kernel(
    x_hbm, gate_hbm, k_hbm, v_hbm, wq_hbm, wo_hbm, ckv_hbm,
    bwq_hbm, bwuk_hbm, bwuv_hbm, bwo_hbm,
    out_hbm,
    x_ref, gate_ref, out_ref, ring,
    wq_v, wo_v, ckv_v, bwq_v, bwuk_v, bwuv_v, bwo_v,
    ebig, qa_ref, qb_ref, y_ref, sb_ref, gmix_ref, bmix_ref,
    s_buf, m_ref, l_ref, acc_ref, outa_ref,
    ring_sems, w_sems,
):
    NR, S, DH = k_hbm.shape
    NB = ckv_hbm.shape[0]
    H = NR // NB
    DM = x_ref.shape[-1]
    DC = ckv_hbm.shape[-1]
    scale = DH ** -0.5

    GH = _GH
    NG = NR // GH
    KB = ring.shape[2]
    NBATCH = S // KB
    CR = _CHUNK_BYTES // (2 * DH)
    L = _NSLOT
    SCH = _STREAM_BYTES // _CHUNK_BYTES
    TW = 128
    TH = TW * H

    def row_of(g, hh):
        return hh * NG + g

    def b_streams(name):
        src, dst = {
            "bwq": (bwq_hbm, bwq_v), "bwuk": (bwuk_hbm, bwuk_v), "bwuv": (bwuv_hbm, bwuv_v),
            "wq": (wq_hbm, wq_v), "wo": (wo_hbm, wo_v), "bwo": (bwo_hbm, bwo_v),
            "ckv0": (ckv_hbm.at[0], ckv_v.at[0]), "ckv1": (ckv_hbm.at[1], ckv_v.at[1]),
        }[name]
        sem = w_sems.at[_SEM[name]]
        cols = min(src.shape[1], _CHUNK_BYTES // (2 * 16))
        rows = _CHUNK_BYTES // (2 * cols)
        ncb = src.shape[1] // cols
        srows = (SCH // ncb) * rows

        def mk(s):
            def cp(j):
                if ncb == 1:
                    idx = (_ds(s * srows + j * rows, rows),)
                else:
                    idx = (_ds(s * srows + (j // ncb) * rows, rows), _ds((j % ncb) * cols, cols))
                return pltpu.make_async_copy(src.at[idx], dst.at[idx], sem)
            return cp
        return [mk(s) for s in range(src.shape[0] // srows)]

    def b_batches(*names):
        streams = [cp for name in names for cp in b_streams(name)]
        jb = _NDESC // len(streams)

        def mk(j0):
            def run():
                def body(j, c):
                    for i, cp in enumerate(streams):
                        cp(j).start(priority=i % 2)
                    return c
                lax.fori_loop(j0, j0 + jb, body, 0)
            return run
        return [mk(j0) for j0 in range(0, SCH, jb)]

    def wait_all(ref, name):
        pltpu.make_async_copy(ref, ref, w_sems.at[_SEM[name]]).wait()

    def issue_kv(src, g, b, slot):
        for j in range(KB // CR):
            for hh in range(GH):
                pltpu.make_async_copy(
                    src.at[row_of(g, hh), _ds(b * KB + j * CR, CR)],
                    ring.at[slot, hh, pl.ds(j * CR, CR)],
                    ring_sems.at[slot],
                ).start(priority=hh % 2)

    def wait_kv(slot):
        pltpu.make_async_copy(ring.at[slot], ring.at[slot], ring_sems.at[slot]).wait()

    x_cp = pltpu.make_async_copy(x_hbm, x_ref, w_sems.at[_SEM["x"]])
    gate_cp = pltpu.make_async_copy(gate_hbm, gate_ref, w_sems.at[_SEM["gate"]])
    out_cp = pltpu.make_async_copy(out_ref, out_hbm, w_sems.at[_SEM["out"]])

    diag128 = ((_iota((NR, TW), 1) % H) == (_iota((NR, TW), 0) % H)).astype(_F32)
    diag = jnp.tile(diag128, (1, TH // TW))
    row_h = _iota((NR, DH), 0) % H

    def x_rows():
        xv = x_ref[...]
        return jnp.concatenate(
            [jnp.broadcast_to(xv[b:b + 1, :], (H, DM)) for b in range(NB)], axis=0)

    def heads_to_rows(a, w_ref, js):
        acc = None
        for j in js:
            aexp = _dot(a[:, j * TW:(j + 1) * TW], ebig[...])
            lhs = (aexp * diag).astype(_BF16)
            part = _dot(lhs, w_ref[j * TH:(j + 1) * TH, :])
            acc = part if acc is None else acc + part
        return acc

    def tiles(n, half):
        return range(half * (n // 2), (half + 1) * (n // 2))

    def p_const():
        ebig[...] = ((_iota((TW, TH), 1) // H) == _iota((TW, TH), 0)).astype(_BF16)
        x_cp.wait()
        gate_cp.wait()

    def p_gate():
        row8 = _iota((8, DM), 0)
        xv = x_ref[...].astype(_F32)
        x8 = jnp.zeros((8, DM), _F32)
        for b in range(NB):
            x8 = jnp.where(row8 == b, xv[b:b + 1, :], x8)
        gate = jax.nn.sigmoid(jnp.sum(
            x8 * gate_ref[...].astype(_F32).reshape(1, DM), axis=-1, keepdims=True))
        gmix_ref[...] = jnp.broadcast_to(gate, (8, DM))
        outa_ref[...] = jnp.zeros((8, DM), _F32)

    def p_aq():
        wait_all(wq_v, "wq")
        t = _dot(x_rows(), wq_v[...])
        qa = jnp.zeros((NR, DH), _F32)
        for u in range(H):
            qa = jnp.where(row_h == u, t[:, u * DH:(u + 1) * DH], qa)
        qa_ref[...] = qa.astype(_BF16).astype(_F32)

    def p_bq(half):
        def run():
            if half == 0:
                wait_all(bwq_v, "bwq")
            part = heads_to_rows(x_rows(), bwq_v, tiles(DM // TW, half))
            qb_ref[...] = part if half == 0 else qb_ref[...] + part
        return run

    def p_by(half):
        def run():
            if half == 0:
                wait_all(bwuk_v, "bwuk")
            qb = qb_ref[...].astype(_BF16)
            for j in tiles(DC // TW, half):
                tt = _dot_nt(qb, bwuk_v[j * TH:(j + 1) * TH, :])
                tm = (tt * diag).astype(_BF16)
                y_ref[:, j * TW:(j + 1) * TW] = _dot_nt(tm, ebig[...])
        return run

    def p_scores(b, half):
        def run():
            if half == 0:
                wait_all(ckv_v.at[b], "ckv%d" % b)
            yb = y_ref[b * H:(b + 1) * H, :].astype(_BF16)
            ks = slice(half * (S // 2), (half + 1) * (S // 2))
            sb_ref[:, ks] = _dot_nt(yb, ckv_v[b, ks, :]) * scale
        return run

    def p_softmax(b):
        def run():
            s = sb_ref[...]
            m = jnp.max(s, axis=-1, keepdims=True)
            p = jnp.exp(s - m)
            sb_ref[...] = p / jnp.sum(p, axis=-1, keepdims=True)
        return run

    def p_ctx(b):
        def run():
            y_ref[b * H:(b + 1) * H, :] = _dot(sb_ref[...].astype(_BF16), ckv_v[b])
        return run

    def p_buv(half):
        def run():
            if half == 0:
                wait_all(bwuv_v, "bwuv")
            part = heads_to_rows(y_ref[...].astype(_BF16), bwuv_v, tiles(DC // TW, half))
            qb_ref[...] = part if half == 0 else qb_ref[...] + part
        return run

    def p_bo():
        wait_all(bwo_v, "bwo")
        ctx_d = qb_ref[...].astype(_BF16).astype(_F32)
        lz = jnp.concatenate(
            [jnp.where(row_h == u, ctx_d, 0.0) for u in range(H)], axis=1).astype(_BF16)
        zb = _dot(lz, bwo_v[...])
        row8 = _iota((8, DM), 0)
        out_b = jnp.zeros((8, DM), _F32)
        for b in range(NB):
            sb = jnp.sum(zb[b * H:(b + 1) * H, :], axis=0, keepdims=True)
            out_b = jnp.where(row8 == b, sb, out_b)
        bmix_ref[...] = out_b

    def p_wo():
        wait_all(wo_v, "wo")

    NLT = KB // DH

    def lane_tiles(a):
        return [a[:, t * DH:(t + 1) * DH] for t in range(NLT)]

    def k_begin():
        m_ref[...] = jnp.full(m_ref.shape, -jnp.inf, _F32)

    def k_unit(g, b, slot):
        for hh in range(GH):
            q = jnp.broadcast_to(qa_ref[pl.ds(row_of(g, hh), 1), :], (8, DH)).astype(_BF16)
            s = _dot_nt(q, ring[slot, hh]) * scale
            s_buf[hh, b] = s
            m = m_ref[hh]
            for t in lane_tiles(s):
                m = jnp.maximum(m, t)
            m_ref[hh] = m

    def v_begin():
        for hh in range(GH):
            m = jnp.max(m_ref[hh], axis=-1, keepdims=True)
            m_ref[hh] = jnp.broadcast_to(m, (8, DH))
        l_ref[...] = jnp.zeros(l_ref.shape, _F32)
        acc_ref[...] = jnp.zeros(acc_ref.shape, _F32)

    def v_probs(b):
        ps = []
        for hh in range(GH):
            p = jnp.exp(s_buf[hh, b] - jnp.tile(m_ref[hh], (1, NLT)))
            l = l_ref[hh]
            for t in lane_tiles(p):
                l = l + t
            l_ref[hh] = l
            ps.append(p.astype(_BF16))
        return ps

    def v_unit(b, slot):
        ps = v_probs(b)
        wait_kv(slot)
        for hh in range(GH):
            acc_ref[hh] = acc_ref[hh] + _dot(ps[hh], ring[slot, hh])

    def inv_row_sums():
        return [1.0 / jnp.sum(l_ref[hh], axis=-1, keepdims=True) for hh in range(GH)]

    def finish_heads(g, accs, inv_ls):
        row8d = _iota((8, DH), 0)
        out = outa_ref[...]
        for hh in range(GH):
            r = row_of(g, hh)
            o = jnp.where(row8d == r // H, accs[hh] * inv_ls[hh], 0.0).astype(_BF16)
            out = out + _dot(o, wo_v[_ds((r % H) * DH, DH), :])
        outa_ref[...] = out

    def v_last_unit_fused(g, slot):
        ps = v_probs(NBATCH - 1)
        inv_ls = inv_row_sums()
        wait_kv(slot)
        accs = [acc_ref[hh] + _dot(ps[hh], ring[slot, hh]) for hh in range(GH)]
        finish_heads(g, accs, inv_ls)

    for i, run in enumerate(b_batches("wq", "wo")):
        run()
        if i == 0:
            x_cp.start(priority=0)
            gate_cp.start(priority=1)
    pro = [p_const, p_gate, p_aq]
    for u in range(L):
        issue_kv(k_hbm, 0, u, u % L)
        if u < len(pro):
            pro[u]()
    for piece in pro[L:]:
        piece()

    extras = {}

    def attach(u, fn):
        extras.setdefault(u, []).append(fn)

    u = 0
    loaded = {}
    for names in (("bwq", "bwo", "bwuk", "bwuv"), ("ckv0", "ckv1")):
        for run in b_batches(*names):
            attach(u, run)
            u += 1
        for name in names:
            loaded[name] = u

    def chain(u, pieces):
        for piece in pieces:
            attach(u, piece)
            u += 1
        return u

    attach(1, p_wo)
    u = chain(loaded["bwq"] + 1, [p_bq(0), p_bq(1)])
    u = chain(max(u, loaded["bwuk"] + 1), [p_by(0), p_by(1)])
    for b in range(NB):
        u = chain(max(u, loaded["ckv%d" % b] + 1),
                  [p_scores(b, 0), p_scores(b, 1), p_softmax(b), p_ctx(b)])
    u = chain(max(u, loaded["bwuv"] + 1), [p_buv(0), p_buv(1)])
    u = chain(max(u, loaded["bwo"] + 1), [p_bo])
    assert max(extras) < (NG - 1) * 2 * NBATCH

    def run_extras(phase, lo, hi, g, b):
        for uu in sorted(extras):
            eg, ephase, eb = uu // (2 * NBATCH), (uu // NBATCH) % 2, uu % NBATCH
            if ephase == phase and lo <= eb < hi:
                for fn in extras[uu]:
                    pl.when(jnp.logical_and(g == eg, b == eb))(fn)

    def group_body(g, final):
        base = g * (2 * NBATCH)

        def slot_of(u):
            return (base + u) % L

        def refill(src, gg, bb, slot, phase, lo, hi, b):
            issue_kv(src, gg, bb, slot)
            if not final:
                run_extras(phase, lo, hi, g, b)

        k_begin()

        def k_same(b, c):
            wait_kv(slot_of(b))
            k_unit(g, b, slot_of(b))
            refill(k_hbm, g, b + L, slot_of(b), 0, 0, NBATCH - L, b)
            return c
        lax.fori_loop(0, NBATCH - L, k_same, 0)

        def k_next(b, c):
            wait_kv(slot_of(b))
            k_unit(g, b, slot_of(b))
            refill(v_hbm, g, b + L - NBATCH, slot_of(b), 0, NBATCH - L, NBATCH, b)
            return c
        lax.fori_loop(NBATCH - L, NBATCH, k_next, 0)

        v_begin()

        def v_same(b, c):
            v_unit(b, slot_of(NBATCH + b))
            refill(v_hbm, g, b + L, slot_of(NBATCH + b), 1, 0, NBATCH - L, b)
            return c
        lax.fori_loop(0, NBATCH - L, v_same, 0)

        if final:
            def v_drain(b, c):
                v_unit(b, slot_of(NBATCH + b))
                return c
            lax.fori_loop(NBATCH - L, NBATCH - 1, v_drain, 0)
            v_last_unit_fused(g, slot_of(2 * NBATCH - 1))
        else:
            def v_next(b, c):
                v_unit(b, slot_of(NBATCH + b))
                refill(k_hbm, g + 1, b + L - NBATCH, slot_of(NBATCH + b),
                       1, NBATCH - L, NBATCH, b)
                return c
            lax.fori_loop(NBATCH - L, NBATCH, v_next, 0)
            finish_heads(g, [acc_ref[hh] for hh in range(GH)], inv_row_sums())

    def regular_group(g, c):
        group_body(g, False)
        return c
    lax.fori_loop(0, NG - 1, regular_group, 0)
    group_body(NG - 1, True)

    gate = gmix_ref[...]
    res = gate * outa_ref[...] + (1.0 - gate) * bmix_ref[...]
    out_ref[...] = res[0:NB, :].astype(out_ref.dtype)
    out_cp.start()
    out_cp.wait()


@jax.jit
def pallas_gated_mix__mha_block_cached__compressed_kv_cla__decode_kernel(
    A_x: jax.Array,
    A_k_cache: jax.Array,
    A_v_cache: jax.Array,
    A_wq: jax.Array,
    A_wo: jax.Array,
    B_x: jax.Array,
    B_c_kv: jax.Array,
    B_w_q: jax.Array,
    B_w_uk: jax.Array,
    B_w_uv: jax.Array,
    B_w_o: jax.Array,
    gate_w: jax.Array,
):
    del B_x
    B, H, S, DH = A_k_cache.shape
    DM = A_x.shape[-1]
    DC = B_c_kv.shape[-1]
    NR = B * H
    KB = (_NDESC * _CHUNK_BYTES) // (_GH * DH * 2)
    assert B == 2 and A_x.shape[1] == 1

    k = A_k_cache.reshape(NR, S, DH)
    v = A_v_cache.reshape(NR, S, DH)
    bwq = B_w_q.reshape(DM * H, DH)
    bwuk = B_w_uk.reshape(DC * H, DH)
    bwuv = B_w_uv.reshape(DC * H, DH)
    bwo = B_w_o.reshape(H * DH, DM)

    hbm = pl.BlockSpec(memory_space=pl.ANY)
    dt = A_k_cache.dtype

    out = pl.pallas_call(
        _kernel,
        out_shape=jax.ShapeDtypeStruct((B, DM), A_x.dtype),
        in_specs=[hbm] * 11,
        out_specs=hbm,
        scratch_shapes=[
            pltpu.VMEM((B, DM), A_x.dtype),
            pltpu.VMEM(gate_w.shape, gate_w.dtype),
            pltpu.VMEM((B, DM), A_x.dtype),
            pltpu.VMEM((_NSLOT, _GH, KB, DH), dt),
            pltpu.VMEM(A_wq.shape, dt),
            pltpu.VMEM(A_wo.shape, dt),
            pltpu.VMEM(B_c_kv.shape, dt),
            pltpu.VMEM(bwq.shape, dt),
            pltpu.VMEM(bwuk.shape, dt),
            pltpu.VMEM(bwuv.shape, dt),
            pltpu.VMEM(bwo.shape, dt),
            pltpu.VMEM((128, 128 * H), _BF16),
            pltpu.VMEM((NR, DH), _F32),
            pltpu.VMEM((NR, DH), _F32),
            pltpu.VMEM((NR, DC), _F32),
            pltpu.VMEM((H, S), _F32),
            pltpu.VMEM((8, DM), _F32),
            pltpu.VMEM((8, DM), _F32),
            pltpu.VMEM((_GH, S // KB, 8, KB), _F32),
            pltpu.VMEM((_GH, 8, DH), _F32),
            pltpu.VMEM((_GH, 8, DH), _F32),
            pltpu.VMEM((_GH, 8, DH), _F32),
            pltpu.VMEM((8, DM), _F32),
            pltpu.SemaphoreType.DMA((_NSLOT,)),
            pltpu.SemaphoreType.DMA((len(_SEM),)),
        ],
        compiler_params=pltpu.CompilerParams(vmem_limit_bytes=100 * 1024 * 1024),
    )(A_x.reshape(B, DM), gate_w, k, v, A_wq, A_wo, B_c_kv, bwq, bwuk, bwuv, bwo)
    return out.reshape(B, 1, DM)
```

```python
import jax
import jax.numpy as jnp
from jax import lax
import jax.experimental.pallas as pl
import jax.experimental.pallas.tpu as pltpu

_NT = (((1,), (1,)), ((), ()))
_F32 = jnp.float32
_BF16 = jnp.bfloat16

_CHUNK_BYTES = 32 * 1024
_NDESC = 64
_GH = 16
_NSLOT = 3
_STREAM_BYTES = 512 * 1024

_SEM = {"bwq": 0, "bwuk": 1, "bwuv": 2, "wq": 3, "wo": 4, "bwo": 5,
        "ckv0": 6, "ckv1": 7, "x": 8, "gate": 9, "out": 10}


def _dot(a, b):
    return jnp.dot(a, b, preferred_element_type=_F32)


def _dot_nt(a, b):
    return lax.dot_general(a, b, _NT, preferred_element_type=_F32)


def _iota(shape, dim):
    return lax.broadcasted_iota(jnp.int32, shape, dim)


def _ds(start, size):
    return pl.ds(pl.multiple_of(start, size), size)


def _kernel(
    x_hbm, gate_hbm, k_hbm, v_hbm, wq_hbm, wo_hbm, ckv_hbm,
    bwq_hbm, bwuk_hbm, bwuv_hbm, bwo_hbm,
    out_hbm,
    x_ref, gate_ref, out_ref, ring,
    wq_v, wo_v, ckv_v, bwq_v, bwuk_v, bwuv_v, bwo_v,
    ebig, qa_ref, qb_ref, y_ref, sb_ref, gmix_ref, bmix_ref,
    s_buf, m_ref, l_ref, acc_ref, outa_ref,
    ring_sems, w_sems,
):
    NR, S, DH = k_hbm.shape
    NB = ckv_hbm.shape[0]
    H = NR // NB
    DM = x_ref.shape[-1]
    DC = ckv_hbm.shape[-1]
    scale = DH ** -0.5

    GH = _GH
    NG = NR // GH
    KB = ring.shape[2]
    NBATCH = S // KB
    CR = _CHUNK_BYTES // (2 * DH)
    L = _NSLOT
    SCH = _STREAM_BYTES // _CHUNK_BYTES
    TW = 128
    TH = TW * H

    def row_of(g, hh):
        return hh * NG + g

    def b_streams(name):
        src, dst = {
            "bwq": (bwq_hbm, bwq_v), "bwuk": (bwuk_hbm, bwuk_v), "bwuv": (bwuv_hbm, bwuv_v),
            "wq": (wq_hbm, wq_v), "wo": (wo_hbm, wo_v), "bwo": (bwo_hbm, bwo_v),
            "ckv0": (ckv_hbm.at[0], ckv_v.at[0]), "ckv1": (ckv_hbm.at[1], ckv_v.at[1]),
        }[name]
        sem = w_sems.at[_SEM[name]]
        cols = min(src.shape[1], _CHUNK_BYTES // (2 * 16))
        rows = _CHUNK_BYTES // (2 * cols)
        ncb = src.shape[1] // cols
        srows = (SCH // ncb) * rows
        assert src.shape[1] % cols == 0 and SCH % ncb == 0 and src.shape[0] % srows == 0

        def mk(s):
            def cp(j):
                if ncb == 1:
                    idx = (_ds(s * srows + j * rows, rows),)
                else:
                    idx = (_ds(s * srows + (j // ncb) * rows, rows), _ds((j % ncb) * cols, cols))
                return pltpu.make_async_copy(src.at[idx], dst.at[idx], sem)
            return cp
        return [mk(s) for s in range(src.shape[0] // srows)]

    def b_batches(*names):
        streams = [cp for name in names for cp in b_streams(name)]
        jb = _NDESC // len(streams)
        assert _NDESC % len(streams) == 0 and SCH % jb == 0

        def mk(j0):
            def run():
                def body(j, c):
                    for i, cp in enumerate(streams):
                        cp(j).start(priority=i % 2)
                    return c
                lax.fori_loop(j0, j0 + jb, body, 0)
            return run
        return [mk(j0) for j0 in range(0, SCH, jb)]

    def wait_all(ref, name):
        pltpu.make_async_copy(ref, ref, w_sems.at[_SEM[name]]).wait()

    def issue_kv(src, g, b, slot):
        for j in range(KB // CR):
            for hh in range(GH):
                pltpu.make_async_copy(
                    src.at[row_of(g, hh), _ds(b * KB + j * CR, CR)],
                    ring.at[slot, hh, pl.ds(j * CR, CR)],
                    ring_sems.at[slot],
                ).start(priority=hh % 2)

    def wait_kv(slot):
        pltpu.make_async_copy(ring.at[slot], ring.at[slot], ring_sems.at[slot]).wait()

    x_cp = pltpu.make_async_copy(x_hbm, x_ref, w_sems.at[_SEM["x"]])
    gate_cp = pltpu.make_async_copy(gate_hbm, gate_ref, w_sems.at[_SEM["gate"]])
    out_cp = pltpu.make_async_copy(out_ref, out_hbm, w_sems.at[_SEM["out"]])

    diag128 = ((_iota((NR, TW), 1) % H) == (_iota((NR, TW), 0) % H)).astype(_F32)
    diag = jnp.tile(diag128, (1, TH // TW))
    row_h = _iota((NR, DH), 0) % H

    def x_rows():
        xv = x_ref[...]
        return jnp.concatenate(
            [jnp.broadcast_to(xv[b:b + 1, :], (H, DM)) for b in range(NB)], axis=0)

    def heads_to_rows(a, w_ref, js):
        acc = None
        for j in js:
            aexp = _dot(a[:, j * TW:(j + 1) * TW], ebig[...])
            lhs = (aexp * diag).astype(_BF16)
            part = _dot(lhs, w_ref[j * TH:(j + 1) * TH, :])
            acc = part if acc is None else acc + part
        return acc

    def tiles(n, half):
        return range(half * (n // 2), (half + 1) * (n // 2))

    def p_const():
        ebig[...] = ((_iota((TW, TH), 1) // H) == _iota((TW, TH), 0)).astype(_BF16)
        x_cp.wait()
        gate_cp.wait()

    def p_gate():
        row8 = _iota((8, DM), 0)
        xv = x_ref[...].astype(_F32)
        x8 = jnp.zeros((8, DM), _F32)
        for b in range(NB):
            x8 = jnp.where(row8 == b, xv[b:b + 1, :], x8)
        gate = jax.nn.sigmoid(jnp.sum(
            x8 * gate_ref[...].astype(_F32).reshape(1, DM), axis=-1, keepdims=True))
        gmix_ref[...] = jnp.broadcast_to(gate, (8, DM))
        outa_ref[...] = jnp.zeros((8, DM), _F32)

    def p_aq():
        wait_all(wq_v, "wq")
        t = _dot(x_rows(), wq_v[...])
        qa = jnp.zeros((NR, DH), _F32)
        for u in range(H):
            qa = jnp.where(row_h == u, t[:, u * DH:(u + 1) * DH], qa)
        qa_ref[...] = qa.astype(_BF16).astype(_F32)

    def p_bq(half):
        def run():
            if half == 0:
                wait_all(bwq_v, "bwq")
            part = heads_to_rows(x_rows(), bwq_v, tiles(DM // TW, half))
            qb_ref[...] = part if half == 0 else qb_ref[...] + part
        return run

    def p_by(half):
        def run():
            if half == 0:
                wait_all(bwuk_v, "bwuk")
            qb = qb_ref[...].astype(_BF16)
            for j in tiles(DC // TW, half):
                tt = _dot_nt(qb, bwuk_v[j * TH:(j + 1) * TH, :])
                tm = (tt * diag).astype(_BF16)
                y_ref[:, j * TW:(j + 1) * TW] = _dot_nt(tm, ebig[...])
        return run

    def p_scores(b, half):
        def run():
            if half == 0:
                wait_all(ckv_v.at[b], "ckv%d" % b)
            yb = y_ref[b * H:(b + 1) * H, :].astype(_BF16)
            ks = slice(half * (S // 2), (half + 1) * (S // 2))
            sb_ref[:, ks] = _dot_nt(yb, ckv_v[b, ks, :]) * scale
        return run

    def p_softmax(b):
        def run():
            s = sb_ref[...]
            m = jnp.max(s, axis=-1, keepdims=True)
            p = jnp.exp(s - m)
            sb_ref[...] = p / jnp.sum(p, axis=-1, keepdims=True)
        return run

    def p_ctx(b):
        def run():
            y_ref[b * H:(b + 1) * H, :] = _dot(sb_ref[...].astype(_BF16), ckv_v[b])
        return run

    def p_buv(half):
        def run():
            if half == 0:
                wait_all(bwuv_v, "bwuv")
            part = heads_to_rows(y_ref[...].astype(_BF16), bwuv_v, tiles(DC // TW, half))
            qb_ref[...] = part if half == 0 else qb_ref[...] + part
        return run

    def p_bo():
        wait_all(bwo_v, "bwo")
        ctx_d = qb_ref[...].astype(_BF16).astype(_F32)
        lz = jnp.concatenate(
            [jnp.where(row_h == u, ctx_d, 0.0) for u in range(H)], axis=1).astype(_BF16)
        zb = _dot(lz, bwo_v[...])
        row8 = _iota((8, DM), 0)
        out_b = jnp.zeros((8, DM), _F32)
        for b in range(NB):
            sb = jnp.sum(zb[b * H:(b + 1) * H, :], axis=0, keepdims=True)
            out_b = jnp.where(row8 == b, sb, out_b)
        bmix_ref[...] = out_b

    def p_wo():
        wait_all(wo_v, "wo")

    NLT = KB // DH

    def lane_tiles(a):
        return [a[:, t * DH:(t + 1) * DH] for t in range(NLT)]

    def k_begin():
        m_ref[...] = jnp.full(m_ref.shape, -jnp.inf, _F32)

    def k_unit(g, b, slot):
        for hh in range(GH):
            q = jnp.broadcast_to(qa_ref[pl.ds(row_of(g, hh), 1), :], (8, DH)).astype(_BF16)
            s = _dot_nt(q, ring[slot, hh]) * scale
            s_buf[hh, b] = s
            m = m_ref[hh]
            for t in lane_tiles(s):
                m = jnp.maximum(m, t)
            m_ref[hh] = m

    def v_begin():
        for hh in range(GH):
            m = jnp.max(m_ref[hh], axis=-1, keepdims=True)
            m_ref[hh] = jnp.broadcast_to(m, (8, DH))
        l_ref[...] = jnp.zeros(l_ref.shape, _F32)
        acc_ref[...] = jnp.zeros(acc_ref.shape, _F32)

    def v_probs(b):
        ps = []
        for hh in range(GH):
            p = jnp.exp(s_buf[hh, b] - jnp.tile(m_ref[hh], (1, NLT)))
            l = l_ref[hh]
            for t in lane_tiles(p):
                l = l + t
            l_ref[hh] = l
            ps.append(p.astype(_BF16))
        return ps

    def v_unit(b, slot):
        ps = v_probs(b)
        wait_kv(slot)
        for hh in range(GH):
            acc_ref[hh] = acc_ref[hh] + _dot(ps[hh], ring[slot, hh])

    def inv_row_sums():
        return [1.0 / jnp.sum(l_ref[hh], axis=-1, keepdims=True) for hh in range(GH)]

    def finish_heads(g, accs, inv_ls):
        row8d = _iota((8, DH), 0)
        out = outa_ref[...]
        for hh in range(GH):
            r = row_of(g, hh)
            o = jnp.where(row8d == r // H, accs[hh] * inv_ls[hh], 0.0).astype(_BF16)
            out = out + _dot(o, wo_v[_ds((r % H) * DH, DH), :])
        outa_ref[...] = out

    def v_last_unit_fused(g, slot):
        ps = v_probs(NBATCH - 1)
        inv_ls = inv_row_sums()
        wait_kv(slot)
        accs = [acc_ref[hh] + _dot(ps[hh], ring[slot, hh]) for hh in range(GH)]
        finish_heads(g, accs, inv_ls)

    for i, run in enumerate(b_batches("wq", "wo")):
        run()
        if i == 0:
            x_cp.start(priority=0)
            gate_cp.start(priority=1)
    pro = [p_const, p_gate, p_aq]
    for u in range(L):
        issue_kv(k_hbm, 0, u, u % L)
        if u < len(pro):
            pro[u]()
    for piece in pro[L:]:
        piece()

    extras = {}

    def attach(u, fn):
        extras.setdefault(u, []).append(fn)

    u = 0
    loaded = {}
    for names in (("bwq", "bwo", "bwuk", "bwuv"), ("ckv0", "ckv1")):
        for run in b_batches(*names):
            attach(u, run)
            u += 1
        for name in names:
            loaded[name] = u

    def chain(u, pieces):
        for piece in pieces:
            attach(u, piece)
            u += 1
        return u

    attach(1, p_wo)
    u = chain(loaded["bwq"] + 1, [p_bq(0), p_bq(1)])
    u = chain(max(u, loaded["bwuk"] + 1), [p_by(0), p_by(1)])
    for b in range(NB):
        u = chain(max(u, loaded["ckv%d" % b] + 1),
                  [p_scores(b, 0), p_scores(b, 1), p_softmax(b), p_ctx(b)])
    u = chain(max(u, loaded["bwuv"] + 1), [p_buv(0), p_buv(1)])
    u = chain(max(u, loaded["bwo"] + 1), [p_bo])
    assert max(extras) < (NG - 1) * 2 * NBATCH

    def run_extras(phase, lo, hi, g, b):
        for uu in sorted(extras):
            eg, ephase, eb = uu // (2 * NBATCH), (uu // NBATCH) % 2, uu % NBATCH
            if ephase == phase and lo <= eb < hi:
                for fn in extras[uu]:
                    pl.when(jnp.logical_and(g == eg, b == eb))(fn)

    def group_body(g, final):
        base = g * (2 * NBATCH)

        def slot_of(u):
            return (base + u) % L

        def refill(src, gg, bb, slot, phase, lo, hi, b):
            issue_kv(src, gg, bb, slot)
            if not final:
                run_extras(phase, lo, hi, g, b)

        k_begin()

        def k_same(b, c):
            wait_kv(slot_of(b))
            k_unit(g, b, slot_of(b))
            refill(k_hbm, g, b + L, slot_of(b), 0, 0, NBATCH - L, b)
            return c
        lax.fori_loop(0, NBATCH - L, k_same, 0)

        def k_next(b, c):
            wait_kv(slot_of(b))
            k_unit(g, b, slot_of(b))
            refill(v_hbm, g, b + L - NBATCH, slot_of(b), 0, NBATCH - L, NBATCH, b)
            return c
        lax.fori_loop(NBATCH - L, NBATCH, k_next, 0)

        v_begin()

        def v_same(b, c):
            v_unit(b, slot_of(NBATCH + b))
            refill(v_hbm, g, b + L, slot_of(NBATCH + b), 1, 0, NBATCH - L, b)
            return c
        lax.fori_loop(0, NBATCH - L, v_same, 0)

        if final:
            def v_drain(b, c):
                v_unit(b, slot_of(NBATCH + b))
                return c
            lax.fori_loop(NBATCH - L, NBATCH - 1, v_drain, 0)
            v_last_unit_fused(g, slot_of(2 * NBATCH - 1))
        else:
            def v_next(b, c):
                v_unit(b, slot_of(NBATCH + b))
                refill(k_hbm, g + 1, b + L - NBATCH, slot_of(NBATCH + b),
                       1, NBATCH - L, NBATCH, b)
                return c
            lax.fori_loop(NBATCH - L, NBATCH, v_next, 0)
            finish_heads(g, [acc_ref[hh] for hh in range(GH)], inv_row_sums())

    def regular_group(g, c):
        group_body(g, False)
        return c
    lax.fori_loop(0, NG - 1, regular_group, 0)
    group_body(NG - 1, True)

    gate = gmix_ref[...]
    res = gate * outa_ref[...] + (1.0 - gate) * bmix_ref[...]
    out_ref[...] = res[0:NB, :].astype(out_ref.dtype)
    out_cp.start()
    out_cp.wait()


@jax.jit
def pallas_gated_mix__mha_block_cached__compressed_kv_cla__decode_kernel(
    A_x: jax.Array,
    A_k_cache: jax.Array,
    A_v_cache: jax.Array,
    A_wq: jax.Array,
    A_wo: jax.Array,
    B_x: jax.Array,
    B_c_kv: jax.Array,
    B_w_q: jax.Array,
    B_w_uk: jax.Array,
    B_w_uv: jax.Array,
    B_w_o: jax.Array,
    gate_w: jax.Array,
):
    del B_x
    B, H, S, DH = A_k_cache.shape
    DM = A_x.shape[-1]
    DC = B_c_kv.shape[-1]
    NR = B * H
    KB = (_NDESC * _CHUNK_BYTES) // (_GH * DH * 2)
    assert B == 2 and A_x.shape == (B, 1, DM) and A_v_cache.shape == A_k_cache.shape
    assert A_wq.shape == (DM, H * DH) and A_wo.shape == (H * DH, DM)
    assert B_c_kv.shape == (B, S, DC) and B_w_q.shape == (DM, H, DH)
    assert B_w_uk.shape == B_w_uv.shape == (DC, H, DH) and B_w_o.shape == (H, DH, DM)
    assert DH == 128 and DM % 256 == 0 and DC % 256 == 0 and S % 256 == 0
    assert S % KB == 0 and S // KB > _NSLOT and NR % _GH == 0 and (NR // _GH) * (_GH // B) == H

    k = A_k_cache.reshape(NR, S, DH)
    v = A_v_cache.reshape(NR, S, DH)
    bwq = B_w_q.reshape(DM * H, DH)
    bwuk = B_w_uk.reshape(DC * H, DH)
    bwuv = B_w_uv.reshape(DC * H, DH)
    bwo = B_w_o.reshape(H * DH, DM)

    hbm = pl.BlockSpec(memory_space=pl.ANY)
    dt = A_k_cache.dtype

    out = pl.pallas_call(
        _kernel,
        out_shape=jax.ShapeDtypeStruct((B, DM), A_x.dtype),
        in_specs=[hbm] * 11,
        out_specs=hbm,
        scratch_shapes=[
            pltpu.VMEM((B, DM), A_x.dtype),
            pltpu.VMEM(gate_w.shape, gate_w.dtype),
            pltpu.VMEM((B, DM), A_x.dtype),
            pltpu.VMEM((_NSLOT, _GH, KB, DH), dt),
            pltpu.VMEM(A_wq.shape, dt),
            pltpu.VMEM(A_wo.shape, dt),
            pltpu.VMEM(B_c_kv.shape, dt),
            pltpu.VMEM(bwq.shape, dt),
            pltpu.VMEM(bwuk.shape, dt),
            pltpu.VMEM(bwuv.shape, dt),
            pltpu.VMEM(bwo.shape, dt),
            pltpu.VMEM((128, 128 * H), _BF16),
            pltpu.VMEM((NR, DH), _F32),
            pltpu.VMEM((NR, DH), _F32),
            pltpu.VMEM((NR, DC), _F32),
            pltpu.VMEM((H, S), _F32),
            pltpu.VMEM((8, DM), _F32),
            pltpu.VMEM((8, DM), _F32),
            pltpu.VMEM((_GH, S // KB, 8, KB), _F32),
            pltpu.VMEM((_GH, 8, DH), _F32),
            pltpu.VMEM((_GH, 8, DH), _F32),
            pltpu.VMEM((_GH, 8, DH), _F32),
            pltpu.VMEM((8, DM), _F32),
            pltpu.SemaphoreType.DMA((_NSLOT,)),
            pltpu.SemaphoreType.DMA((len(_SEM),)),
        ],
        compiler_params=pltpu.CompilerParams(vmem_limit_bytes=100 * 1024 * 1024),
    )(A_x.reshape(B, DM), gate_w, k, v, A_wq, A_wo, B_c_kv, bwq, bwuk, bwuv, bwo)
    return out.reshape(B, 1, DM)
```

```python
import jax
import jax.numpy as jnp
from jax import lax
import jax.experimental.pallas as pl
import jax.experimental.pallas.tpu as pltpu

_NT = (((1,), (1,)), ((), ()))
_F32 = jnp.float32
_BF16 = jnp.bfloat16

_CHUNK_BYTES = 32 * 1024
_NDESC = 64
_GH = 16
_NSLOT = 3
_STREAM_BYTES = 512 * 1024

_SEM = {"bwq": 0, "bwuk": 1, "bwuv": 2, "wq": 3, "wo": 4, "bwo": 5,
        "ckv0": 6, "ckv1": 7, "x": 8, "gate": 9, "out": 10}


def _dot(a, b):
    return jnp.dot(a, b, preferred_element_type=_F32)


def _dot_nt(a, b):
    return lax.dot_general(a, b, _NT, preferred_element_type=_F32)


def _iota(shape, dim):
    return lax.broadcasted_iota(jnp.int32, shape, dim)


def _ds(start, size):
    return pl.ds(pl.multiple_of(start, size), size)


def _kernel(
    x_hbm, gate_hbm, k_hbm, v_hbm, wq_hbm, wo_hbm, ckv_hbm,
    bwq_hbm, bwuk_hbm, bwuv_hbm, bwo_hbm,
    out_hbm,
    x_ref, gate_ref, out_ref, ring,
    wq_v, wo_v, ckv_v, bwq_v, bwuk_v, bwuv_v, bwo_v,
    ebig, qa_ref, qb_ref, y_ref, sb_ref, gmix_ref, bmix_ref,
    s_buf, m_ref, l_ref, acc_ref, outa_ref,
    ring_sems, last_sem, w_sems,
):
    NR, S, DH = k_hbm.shape
    NB = ckv_hbm.shape[0]
    H = NR // NB
    DM = x_ref.shape[-1]
    DC = ckv_hbm.shape[-1]
    scale = DH ** -0.5

    GH = _GH
    NG = NR // GH
    KB = ring.shape[2]
    NBATCH = S // KB
    CR = _CHUNK_BYTES // (2 * DH)
    L = _NSLOT
    SCH = _STREAM_BYTES // _CHUNK_BYTES
    TW = 128
    TH = TW * H

    def row_of(g, hh):
        return hh * NG + g

    def b_streams(name):
        src, dst = {
            "bwq": (bwq_hbm, bwq_v), "bwuk": (bwuk_hbm, bwuk_v), "bwuv": (bwuv_hbm, bwuv_v),
            "wq": (wq_hbm, wq_v), "wo": (wo_hbm, wo_v), "bwo": (bwo_hbm, bwo_v),
            "ckv0": (ckv_hbm.at[0], ckv_v.at[0]), "ckv1": (ckv_hbm.at[1], ckv_v.at[1]),
        }[name]
        sem = w_sems.at[_SEM[name]]
        cols = min(src.shape[1], _CHUNK_BYTES // (2 * 16))
        rows = _CHUNK_BYTES // (2 * cols)
        ncb = src.shape[1] // cols
        srows = (SCH // ncb) * rows
        assert src.shape[1] % cols == 0 and SCH % ncb == 0 and src.shape[0] % srows == 0

        def mk(s):
            def cp(j):
                if ncb == 1:
                    idx = (_ds(s * srows + j * rows, rows),)
                else:
                    idx = (_ds(s * srows + (j // ncb) * rows, rows), _ds((j % ncb) * cols, cols))
                return pltpu.make_async_copy(src.at[idx], dst.at[idx], sem)
            return cp
        return [mk(s) for s in range(src.shape[0] // srows)]

    def b_batches(*names):
        streams = [cp for name in names for cp in b_streams(name)]
        jb = _NDESC // len(streams)
        assert _NDESC % len(streams) == 0 and SCH % jb == 0

        def mk(j0):
            def run():
                def body(j, c):
                    for i, cp in enumerate(streams):
                        cp(j).start(priority=i % 2)
                    return c
                lax.fori_loop(j0, j0 + jb, body, 0)
            return run
        return [mk(j0) for j0 in range(0, SCH, jb)]

    def wait_all(ref, name):
        pltpu.make_async_copy(ref, ref, w_sems.at[_SEM[name]]).wait()

    def issue_kv(src, g, b, slot):
        for j in range(KB // CR):
            for hh in range(GH):
                pltpu.make_async_copy(
                    src.at[row_of(g, hh), _ds(b * KB + j * CR, CR)],
                    ring.at[slot, hh, pl.ds(j * CR, CR)],
                    ring_sems.at[slot],
                ).start(priority=hh % 2)

    KS = KB - CR

    def issue_v_final(g, slot):
        b = NBATCH - 1
        for j in range(KB // CR):
            for hh in range(GH):
                pltpu.make_async_copy(
                    v_hbm.at[row_of(g, hh), pl.ds(b * KB + j * CR, CR)],
                    ring.at[slot, hh, pl.ds(j * CR, CR)],
                    ring_sems.at[slot] if j * CR < KS else last_sem.at[0],
                ).start(priority=hh % 2)

    def wait_kv(slot):
        pltpu.make_async_copy(ring.at[slot], ring.at[slot], ring_sems.at[slot]).wait()

    x_cp = pltpu.make_async_copy(x_hbm, x_ref, w_sems.at[_SEM["x"]])
    gate_cp = pltpu.make_async_copy(gate_hbm, gate_ref, w_sems.at[_SEM["gate"]])
    out_cp = pltpu.make_async_copy(out_ref, out_hbm, w_sems.at[_SEM["out"]])

    diag128 = ((_iota((NR, TW), 1) % H) == (_iota((NR, TW), 0) % H)).astype(_F32)
    diag = jnp.tile(diag128, (1, TH // TW))
    row_h = _iota((NR, DH), 0) % H

    def x_rows():
        xv = x_ref[...]
        return jnp.concatenate(
            [jnp.broadcast_to(xv[b:b + 1, :], (H, DM)) for b in range(NB)], axis=0)

    def heads_to_rows(a, w_ref, js):
        acc = None
        for j in js:
            aexp = _dot(a[:, j * TW:(j + 1) * TW], ebig[...])
            lhs = (aexp * diag).astype(_BF16)
            part = _dot(lhs, w_ref[j * TH:(j + 1) * TH, :])
            acc = part if acc is None else acc + part
        return acc

    def tiles(n, half):
        return range(half * (n // 2), (half + 1) * (n // 2))

    def p_const():
        ebig[...] = ((_iota((TW, TH), 1) // H) == _iota((TW, TH), 0)).astype(_BF16)
        x_cp.wait()
        gate_cp.wait()

    def p_gate():
        row8 = _iota((8, DM), 0)
        xv = x_ref[...].astype(_F32)
        x8 = jnp.zeros((8, DM), _F32)
        for b in range(NB):
            x8 = jnp.where(row8 == b, xv[b:b + 1, :], x8)
        gate = jax.nn.sigmoid(jnp.sum(
            x8 * gate_ref[...].astype(_F32).reshape(1, DM), axis=-1, keepdims=True))
        gmix_ref[...] = jnp.broadcast_to(gate, (8, DM))
        outa_ref[...] = jnp.zeros((8, DM), _F32)

    def p_aq():
        wait_all(wq_v, "wq")
        t = _dot(x_rows(), wq_v[...])
        qa = jnp.zeros((NR, DH), _F32)
        for u in range(H):
            qa = jnp.where(row_h == u, t[:, u * DH:(u + 1) * DH], qa)
        qa_ref[...] = qa.astype(_BF16).astype(_F32)

    def p_bq(half):
        def run():
            if half == 0:
                wait_all(bwq_v, "bwq")
            part = heads_to_rows(x_rows(), bwq_v, tiles(DM // TW, half))
            qb_ref[...] = part if half == 0 else qb_ref[...] + part
        return run

    def p_by(half):
        def run():
            if half == 0:
                wait_all(bwuk_v, "bwuk")
            qb = qb_ref[...].astype(_BF16)
            for j in tiles(DC // TW, half):
                tt = _dot_nt(qb, bwuk_v[j * TH:(j + 1) * TH, :])
                tm = (tt * diag).astype(_BF16)
                y_ref[:, j * TW:(j + 1) * TW] = _dot_nt(tm, ebig[...])
        return run

    def p_scores(b, half):
        def run():
            if half == 0:
                wait_all(ckv_v.at[b], "ckv%d" % b)
            yb = y_ref[b * H:(b + 1) * H, :].astype(_BF16)
            ks = slice(half * (S // 2), (half + 1) * (S // 2))
            sb_ref[:, ks] = _dot_nt(yb, ckv_v[b, ks, :]) * scale
        return run

    def p_softmax(b):
        def run():
            s = sb_ref[...]
            m = jnp.max(s, axis=-1, keepdims=True)
            p = jnp.exp(s - m)
            sb_ref[...] = p / jnp.sum(p, axis=-1, keepdims=True)
        return run

    def p_ctx(b):
        def run():
            y_ref[b * H:(b + 1) * H, :] = _dot(sb_ref[...].astype(_BF16), ckv_v[b])
        return run

    def p_buv(half):
        def run():
            if half == 0:
                wait_all(bwuv_v, "bwuv")
            part = heads_to_rows(y_ref[...].astype(_BF16), bwuv_v, tiles(DC // TW, half))
            qb_ref[...] = part if half == 0 else qb_ref[...] + part
        return run

    def p_bo():
        wait_all(bwo_v, "bwo")
        ctx_d = qb_ref[...].astype(_BF16).astype(_F32)
        lz = jnp.concatenate(
            [jnp.where(row_h == u, ctx_d, 0.0) for u in range(H)], axis=1).astype(_BF16)
        zb = _dot(lz, bwo_v[...])
        row8 = _iota((8, DM), 0)
        out_b = jnp.zeros((8, DM), _F32)
        for b in range(NB):
            sb = jnp.sum(zb[b * H:(b + 1) * H, :], axis=0, keepdims=True)
            out_b = jnp.where(row8 == b, sb, out_b)
        bmix_ref[...] = out_b

    def p_wo():
        wait_all(wo_v, "wo")

    NLT = KB // DH

    def lane_tiles(a):
        return [a[:, t * DH:(t + 1) * DH] for t in range(NLT)]

    def k_begin():
        m_ref[...] = jnp.full(m_ref.shape, -jnp.inf, _F32)

    def k_unit(g, b, slot):
        for hh in range(GH):
            q = jnp.broadcast_to(qa_ref[pl.ds(row_of(g, hh), 1), :], (8, DH)).astype(_BF16)
            s = _dot_nt(q, ring[slot, hh]) * scale
            s_buf[hh, b] = s
            m = m_ref[hh]
            for t in lane_tiles(s):
                m = jnp.maximum(m, t)
            m_ref[hh] = m

    def v_begin():
        for hh in range(GH):
            m = jnp.max(m_ref[hh], axis=-1, keepdims=True)
            m_ref[hh] = jnp.broadcast_to(m, (8, DH))
        l_ref[...] = jnp.zeros(l_ref.shape, _F32)
        acc_ref[...] = jnp.zeros(acc_ref.shape, _F32)

    def v_probs(b):
        ps = []
        for hh in range(GH):
            p = jnp.exp(s_buf[hh, b] - jnp.tile(m_ref[hh], (1, NLT)))
            l = l_ref[hh]
            for t in lane_tiles(p):
                l = l + t
            l_ref[hh] = l
            ps.append(p.astype(_BF16))
        return ps

    def v_unit(b, slot):
        ps = v_probs(b)
        wait_kv(slot)
        for hh in range(GH):
            acc_ref[hh] = acc_ref[hh] + _dot(ps[hh], ring[slot, hh])

    def inv_row_sums():
        return [1.0 / jnp.sum(l_ref[hh], axis=-1, keepdims=True) for hh in range(GH)]

    def finish_heads(g, accs, inv_ls):
        row8d = _iota((8, DH), 0)
        out = outa_ref[...]
        for i in range(GH // NB):
            o = jnp.zeros((8, DH), _F32)
            for b in range(NB):
                hh = i + b * (GH // NB)
                o = jnp.where(row8d == b, accs[hh] * inv_ls[hh], o)
            h = row_of(g, i)
            out = out + _dot(o.astype(_BF16), wo_v[_ds(h * DH, DH), :])
        outa_ref[...] = out

    def v_last_unit_fused(g, slot):
        ps = v_probs(NBATCH - 1)
        inv_ls = inv_row_sums()
        head = ring.at[slot, :, pl.ds(0, KS)]
        pltpu.make_async_copy(head, head, ring_sems.at[slot]).wait()
        accs = [acc_ref[hh] + _dot(ps[hh][:, :KS], ring[slot, hh, :KS, :]) for hh in range(GH)]
        last = ring.at[slot, :, pl.ds(KS, CR)]
        pltpu.make_async_copy(last, last, last_sem.at[0]).wait()
        accs = [accs[hh] + _dot(ps[hh][:, KS:], ring[slot, hh, KS:, :]) for hh in range(GH)]
        finish_heads(g, accs, inv_ls)

    for i, run in enumerate(b_batches("wq", "wo")):
        run()
        if i == 0:
            x_cp.start(priority=0)
            gate_cp.start(priority=1)
    pro = [p_const, p_gate, p_aq]
    for u in range(L):
        issue_kv(k_hbm, 0, u, u % L)
        if u < len(pro):
            pro[u]()
    for piece in pro[L:]:
        piece()

    extras = {}

    def attach(u, fn):
        extras.setdefault(u, []).append(fn)

    u = 0
    loaded = {}
    for names in (("bwq", "bwo", "bwuk", "bwuv"), ("ckv0", "ckv1")):
        for run in b_batches(*names):
            attach(u, run)
            u += 1
        for name in names:
            loaded[name] = u

    def chain(u, pieces):
        for piece in pieces:
            attach(u, piece)
            u += 1
        return u

    attach(1, p_wo)
    u = chain(loaded["bwq"] + 1, [p_bq(0), p_bq(1)])
    u = chain(max(u, loaded["bwuk"] + 1), [p_by(0), p_by(1)])
    for b in range(NB):
        u = chain(max(u, loaded["ckv%d" % b] + 1),
                  [p_scores(b, 0), p_scores(b, 1), p_softmax(b), p_ctx(b)])
    u = chain(max(u, loaded["bwuv"] + 1), [p_buv(0), p_buv(1)])
    u = chain(max(u, loaded["bwo"] + 1), [p_bo])
    assert max(extras) < (NG - 1) * 2 * NBATCH

    def run_extras(phase, lo, hi, g, b):
        for uu in sorted(extras):
            eg, ephase, eb = uu // (2 * NBATCH), (uu // NBATCH) % 2, uu % NBATCH
            if ephase == phase and lo <= eb < hi:
                for fn in extras[uu]:
                    pl.when(jnp.logical_and(g == eg, b == eb))(fn)

    def group_body(g, final):
        base = g * (2 * NBATCH)

        def slot_of(u):
            return (base + u) % L

        def refill(src, gg, bb, slot, phase, lo, hi, b):
            issue_kv(src, gg, bb, slot)
            if not final:
                run_extras(phase, lo, hi, g, b)

        k_begin()

        def k_same(b, c):
            wait_kv(slot_of(b))
            k_unit(g, b, slot_of(b))
            refill(k_hbm, g, b + L, slot_of(b), 0, 0, NBATCH - L, b)
            return c
        lax.fori_loop(0, NBATCH - L, k_same, 0)

        def k_next(b, c):
            wait_kv(slot_of(b))
            k_unit(g, b, slot_of(b))
            refill(v_hbm, g, b + L - NBATCH, slot_of(b), 0, NBATCH - L, NBATCH, b)
            return c
        lax.fori_loop(NBATCH - L, NBATCH, k_next, 0)

        v_begin()

        def v_same(b, c):
            v_unit(b, slot_of(NBATCH + b))
            refill(v_hbm, g, b + L, slot_of(NBATCH + b), 1, 0, NBATCH - L, b)
            return c
        if final:
            n = NBATCH - L - 1
            lax.fori_loop(0, n, v_same, 0)
            v_unit(n, slot_of(NBATCH + n))
            issue_v_final(g, slot_of(NBATCH + n))

            def v_drain(b, c):
                v_unit(b, slot_of(NBATCH + b))
                return c
            lax.fori_loop(NBATCH - L, NBATCH - 1, v_drain, 0)
            v_last_unit_fused(g, slot_of(2 * NBATCH - 1))
        else:
            lax.fori_loop(0, NBATCH - L, v_same, 0)

            def v_next(b, c):
                v_unit(b, slot_of(NBATCH + b))
                refill(k_hbm, g + 1, b + L - NBATCH, slot_of(NBATCH + b),
                       1, NBATCH - L, NBATCH, b)
                return c
            lax.fori_loop(NBATCH - L, NBATCH, v_next, 0)
            finish_heads(g, [acc_ref[hh] for hh in range(GH)], inv_row_sums())

    def regular_group(g, c):
        group_body(g, False)
        return c
    lax.fori_loop(0, NG - 1, regular_group, 0)
    group_body(NG - 1, True)

    gate = gmix_ref[...]
    res = gate * outa_ref[...] + (1.0 - gate) * bmix_ref[...]
    out_ref[...] = res[0:NB, :].astype(out_ref.dtype)
    out_cp.start()
    out_cp.wait()


@jax.jit
def pallas_gated_mix__mha_block_cached__compressed_kv_cla__decode_kernel(
    A_x: jax.Array,
    A_k_cache: jax.Array,
    A_v_cache: jax.Array,
    A_wq: jax.Array,
    A_wo: jax.Array,
    B_x: jax.Array,
    B_c_kv: jax.Array,
    B_w_q: jax.Array,
    B_w_uk: jax.Array,
    B_w_uv: jax.Array,
    B_w_o: jax.Array,
    gate_w: jax.Array,
):
    del B_x
    B, H, S, DH = A_k_cache.shape
    DM = A_x.shape[-1]
    DC = B_c_kv.shape[-1]
    NR = B * H
    KB = (_NDESC * _CHUNK_BYTES) // (_GH * DH * 2)
    assert B == 2 and A_x.shape == (B, 1, DM) and A_v_cache.shape == A_k_cache.shape
    assert A_wq.shape == (DM, H * DH) and A_wo.shape == (H * DH, DM)
    assert B_c_kv.shape == (B, S, DC) and B_w_q.shape == (DM, H, DH)
    assert B_w_uk.shape == B_w_uv.shape == (DC, H, DH) and B_w_o.shape == (H, DH, DM)
    assert DH == 128 and DM % 256 == 0 and DC % 256 == 0 and S % 256 == 0
    assert S % KB == 0 and S // KB > _NSLOT and NR % _GH == 0 and (NR // _GH) * (_GH // B) == H

    k = A_k_cache.reshape(NR, S, DH)
    v = A_v_cache.reshape(NR, S, DH)
    bwq = B_w_q.reshape(DM * H, DH)
    bwuk = B_w_uk.reshape(DC * H, DH)
    bwuv = B_w_uv.reshape(DC * H, DH)
    bwo = B_w_o.reshape(H * DH, DM)

    hbm = pl.BlockSpec(memory_space=pl.ANY)
    dt = A_k_cache.dtype

    out = pl.pallas_call(
        _kernel,
        out_shape=jax.ShapeDtypeStruct((B, DM), A_x.dtype),
        in_specs=[hbm] * 11,
        out_specs=hbm,
        scratch_shapes=[
            pltpu.VMEM((B, DM), A_x.dtype),
            pltpu.VMEM(gate_w.shape, gate_w.dtype),
            pltpu.VMEM((B, DM), A_x.dtype),
            pltpu.VMEM((_NSLOT, _GH, KB, DH), dt),
            pltpu.VMEM(A_wq.shape, dt),
            pltpu.VMEM(A_wo.shape, dt),
            pltpu.VMEM(B_c_kv.shape, dt),
            pltpu.VMEM(bwq.shape, dt),
            pltpu.VMEM(bwuk.shape, dt),
            pltpu.VMEM(bwuv.shape, dt),
            pltpu.VMEM(bwo.shape, dt),
            pltpu.VMEM((128, 128 * H), _BF16),
            pltpu.VMEM((NR, DH), _F32),
            pltpu.VMEM((NR, DH), _F32),
            pltpu.VMEM((NR, DC), _F32),
            pltpu.VMEM((H, S), _F32),
            pltpu.VMEM((8, DM), _F32),
            pltpu.VMEM((8, DM), _F32),
            pltpu.VMEM((_GH, S // KB, 8, KB), _F32),
            pltpu.VMEM((_GH, 8, DH), _F32),
            pltpu.VMEM((_GH, 8, DH), _F32),
            pltpu.VMEM((_GH, 8, DH), _F32),
            pltpu.VMEM((8, DM), _F32),
            pltpu.SemaphoreType.DMA((_NSLOT,)),
            pltpu.SemaphoreType.DMA((1,)),
            pltpu.SemaphoreType.DMA((len(_SEM),)),
        ],
        compiler_params=pltpu.CompilerParams(vmem_limit_bytes=100 * 1024 * 1024),
    )(A_x.reshape(B, DM), gate_w, k, v, A_wq, A_wo, B_c_kv, bwq, bwuk, bwuv, bwo)
    return out.reshape(B, 1, DM)
```
